```python
import jax
import jax.numpy as jnp

def _softmax(x, axis=-1):
    return jax.nn.softmax(x, axis=axis)
def _gelu(x):
    return jax.nn.gelu(x, approximate=True)
def _silu(x):
    return jax.nn.silu(x)
def _sigmoid(x):
    return jax.nn.sigmoid(x)
def _layernorm(x, axis=-1, eps=1e-5):
    m = jnp.mean(x, axis=axis, keepdims=True)
    v = jnp.var(x, axis=axis, keepdims=True)
    return (x - m) / jnp.sqrt(v + eps)
def _scatter_add(tgt, idx, src, axis=0):
    return tgt.at[idx].add(src)
def _segment_sum(src, seg, n):
    return jax.ops.segment_sum(src, seg, n)
class _Rng:
    def __init__(self, key):
        self._k = key
    def _next(self):
        self._k, sub = jax.random.split(self._k)
        return sub
    def normal(self, shape):
        return jax.random.normal(self._next(), shape, dtype=jnp.bfloat16)
    def randint(self, lo, hi, shape):
        return jax.random.randint(self._next(), shape, lo, hi, dtype=jnp.int32)
    def uniform(self, shape, lo=0.0, hi=1.0):
        return jax.random.uniform(self._next(), shape, jnp.bfloat16, lo, hi)
    def permutation(self, n):
        return jax.random.permutation(self._next(), n)


kernel_name = 'gated_mix__ssm_conv_h3__compressed_kv_cla__prompt'

def setup_inputs():
    _rng = _Rng(jax.random.key(int.from_bytes(__import__("os").urandom(4), "little")))
    _w = (lambda a: (lambda t: t.astype(jnp.bfloat16) if jnp.issubdtype(t.dtype, jnp.floating) else t)(jnp.asarray(a)))
    def _A_setup():
        B, S, D = 1, 2048, 1024
        ks = 4
        return {
            "q": _w((lambda *s: _rng.normal(s) * 0.05)(B, S, D)),
            "k": _w((lambda *s: _rng.normal(s) * 0.05)(B, S, D)),
            "v": _w((lambda *s: _rng.normal(s) * 0.05)(B, S, D)),
            "shift_k": _w((lambda *s: _rng.normal(s) * 0.05)(D, ks) * 0.5),
            "ssm_k": _w((lambda *s: _rng.normal(s) * 0.05)(D, S) * (1.0 / S ** 0.5)),
            "ssm_D": _w((lambda *s: _rng.normal(s) * 0.05)(D)),
        }
    _A_in = _A_setup()

    def _B_setup():
        B, H, Sq, Sk, D, M = 1, 32, 2048, 2048, 128, 1024
        Dc = 4 * D
        return {
            "x": _w((lambda *s: _rng.normal(s) * 0.05)(B, Sq, M)),
            "c_kv": _w((lambda *s: _rng.normal(s) * 0.05)(B, Sk, Dc)),
            "w_q": _w((lambda *s: _rng.normal(s) * 0.05)(M, H, D) * (M ** -0.5)),
            "w_uk": _w((lambda *s: _rng.normal(s) * 0.05)(Dc, H, D) * (Dc ** -0.5)),
            "w_uv": _w((lambda *s: _rng.normal(s) * 0.05)(Dc, H, D) * (Dc ** -0.5)),
            "w_o": _w((lambda *s: _rng.normal(s) * 0.05)(H, D, M) * ((H * D) ** -0.5)),
        }
    _B_in = _B_setup()

    return {
        "A_q": _A_in["q"],
        "A_k": _A_in["k"],
        "A_v": _A_in["v"],
        "A_shift_k": _A_in["shift_k"],
        "A_ssm_k": _A_in["ssm_k"],
        "A_ssm_D": _A_in["ssm_D"],
        "B_x": _B_in["x"],
        "B_c_kv": _B_in["c_kv"],
        "B_w_q": _B_in["w_q"],
        "B_w_uk": _B_in["w_uk"],
        "B_w_uv": _B_in["w_uv"],
        "B_w_o": _B_in["w_o"],
        "gate_w": _w((lambda *s: _rng.normal(s) * 0.05)(1024)),
    }

def reference(A_q, A_k, A_v, A_shift_k, A_ssm_k, A_ssm_D, B_x, B_c_kv, B_w_q, B_w_uk, B_w_uv, B_w_o, gate_w):
    def _A_ref(q, k, v, shift_k, ssm_k, ssm_D):
        B, S, D = q.shape
        ks = shift_k.shape[-1]
        k_pad = jnp.pad(k, ((0, 0), (ks - 1, 0), (0, 0)))
        k_shift = jnp.zeros_like(k)
        for t in range(ks):
            k_shift = k_shift + k_pad[:, t:t + S, :] * shift_k[:, ks - 1 - t][None, None, :]
        kv = k_shift * v
        L = 2 * S
        kv_pad = jnp.pad(kv, ((0, 0), (0, S), (0, 0)))
        kf_pad = jnp.pad(ssm_k, ((0, 0), (0, S)))
        kv_f = (lambda x, axes=(-2,-1): jnp.fft.rfft2(x.astype(jnp.float32), axes=axes))(kv_pad[:, None, :, :], axes=(1, 2))
        kf_f = (lambda x, axes=(-2,-1): jnp.fft.rfft2(x.astype(jnp.float32), axes=axes))(kf_pad[:, None, :], axes=(1, 2))
        kf_f = (lambda x, *d: x.transpose(*d))(kf_f, 1, 2, 0)
        y_f = kv_f * kf_f[None, :, :, :]
        y = (lambda x, s, axes=(-2,-1): jnp.fft.irfft2(x, s=s, axes=axes).astype(jnp.bfloat16))(y_f, (1, L), axes=(1, 2))[:, 0, :S, :]
        y = y + kv * ssm_D[None, None, :]
        return q * y

    def _B_ref(x, c_kv, w_q, w_uk, w_uv, w_o):
        B, Sq, M = x.shape[0], x.shape[1], x.shape[2]
        Sk = c_kv.shape[1]
        H, D = w_q.shape[1], w_q.shape[2]
        q = jnp.einsum("bqm,mhd->bhqd", x, w_q)
        k = jnp.einsum("bkc,chd->bhkd", c_kv, w_uk)
        v = jnp.einsum("bkc,chd->bhkd", c_kv, w_uv)
        scores = jnp.einsum("bhqd,bhkd->bhqk", q, k) * (D ** -0.5)
        off = Sk - Sq
        qi = jnp.arange(Sq)[:, None]
        kj = jnp.arange(Sk)[None, :]
        cmask = kj <= (qi + off)
        scores = jnp.where(cmask[None, None], scores, -1e9)
        p = _softmax(scores, axis=-1)
        ctx = jnp.einsum("bhqk,bhkd->bhqd", p, v)
        return jnp.einsum("bhqd,hdm->bqm", ctx, w_o)

    x = A_q
    g = _sigmoid((x * gate_w).sum(-1, keepdims=True))
    a = _A_ref(x, A_k, A_v, A_shift_k, A_ssm_k, A_ssm_D)
    b = _B_ref(x, B_c_kv, B_w_q, B_w_uk, B_w_uv, B_w_o)
    return g * a + (1 - g) * b
```

```python
import os
import functools
import numpy as np
import jax
import jax.numpy as jnp
import jax.experimental.pallas as pl
import jax.experimental.pallas.tpu as pltpu

S, D, H, HD, DC, C = 2048, 1024, 32, 128, 512, 128
NC = S // C
NT = D // 128
NTC = DC // 128
NP = H // 2
BQ = 256
NB = S // BQ
NSUB = BQ // 128
PAD = 8
NPAIR = int(os.environ.get("K_np", NP))
SKIP = int(os.environ.get("K_skip", 64))
MAC_LO = int(os.environ.get("K_maclo", 1))
MAC_HI = int(os.environ.get("K_machi", 12))
DIST = int(os.environ.get("K_dist", 6))
GAP = int(os.environ.get("K_gap", 9))
MLAG = int(os.environ.get("K_mlag", 8))
E_R = int(os.environ.get("K_er", 0))
OD = int(os.environ.get("K_od", 2))
KLAG = int(os.environ.get("K_klag", 6))
XU = int(os.environ.get("K_xu", 14))
XLAG = int(os.environ.get("K_xlag", 5))
MDL = int(os.environ.get("K_mdl", 0))
ENDM = int(os.environ.get("K_endm", 0))
E_Q = int(os.environ.get("K_eq", 3))
NQ = int(os.environ.get("K_nq", 4))
E_MAC = int(os.environ.get("K_emac", 1))
SMEMS = int(os.environ.get("K_sm", 1))
MB = int(os.environ.get("K_mb", 4))
_FL = {"lp": {"XLA_TPU_FORCE_LP_LLO_SCHEDULER": True}, "ev": {"XLA_TPU_EVENLY_DISTRIBUTE_CRITICAL_NODES": True},
       "none": None}
_FLAGS = _FL[os.environ.get("K_fl", "none")]
LOG2E = 1.4426950408889634
QSCALE = (HD ** -0.5) * LOG2E
NEG = -1e9 * LOG2E
BF = jnp.bfloat16
F32 = jnp.float32
U32 = jnp.uint32


def _dft_mats():
    t_nat = np.arange(C, dtype=np.float64)
    t_par = np.concatenate([t_nat[0::2], t_nat[1::2]])
    fk, fx, inv = [], [], []
    for h in range(2):
        f = 2.0 * np.arange(h * C // 2, (h + 1) * C // 2, dtype=np.float64) + 0.5
        for t, dst in ((t_nat, fk), (t_par, fx)):
            ang = 2.0 * np.pi * np.outer(f, t) / (2 * C)
            dst.append(np.concatenate([np.cos(ang), -np.sin(ang)], axis=0))
        ang = 2.0 * np.pi * np.outer(t_par + C, f) / (2 * C)
        inv.append(np.concatenate([np.cos(ang), -np.sin(ang)], axis=1) / C)
    return np.stack([np.stack(fk), np.stack(fx), np.stack(inv)], axis=1).astype(np.float32)


_DFT = _dft_mats()
NT_DIMS = (((1,), (1,)), ((), ()))


def _mm(a, b):
    return jnp.dot(a, b, preferred_element_type=F32)


def _mm_nt(a, b):
    return jax.lax.dot_general(a, b, NT_DIMS, preferred_element_type=F32)


def _ld(ref, idx, lo, hi):
    return pltpu.bitcast(ref[(*idx, slice(lo // 2, hi // 2), slice(None))], BF)


def _lo(w):
    return pltpu.bitcast(w << 16, F32)


def _hi(w):
    return pltpu.bitcast(w & jnp.uint32(0xFFFF0000), F32)


def _emit(mxu_items, vpu_items, skip=0):
    total = sum(cost for cost, _ in mxu_items)
    span = max(total - skip, 1)
    done, k = 0, 0
    for cost, fn in mxu_items:
        fn()
        done += cost
        while k < len(vpu_items) and (k + 1) * span <= (done - skip) * len(vpu_items):
            vpu_items[k]()
            k += 1
    for fn in vpu_items[k:]:
        fn()


def _merge(a, b):
    out, i, k = [], 0, 0
    while i < len(a) or k < len(b):
        if k >= len(b) or (i < len(a) and (i + 1) * len(b) <= (k + 1) * len(a)):
            out.append(a[i])
            i += 1
        else:
            out.append(b[k])
            k += 1
    return out


def _kernel(aq_h, ak_h, av_h, shift_ref, sk_h, ssmd_ref, x_h, c_h, wq_h, wuk_h, wuv_h, wo_h,
            gate_ref, dft_ref, out_h,
            aq, ak, av, sk, x, c, wq_raw, wk_raw, wv_raw, wo, a_buf, acc, out_v,
            shift32, d32, gate32, dft, zero_ref,
            sem_a, sem_x, sem_w, sem_o):
    def a_copies(i):
        cols = pl.ds(i * 128, 128)
        cps = [pltpu.make_async_copy(ak_h.bitcast(U32).at[:, cols], ak.at[i, pl.ds(PAD, S // 2)], sem_a.at[0, i]),
               pltpu.make_async_copy(av_h.bitcast(U32).at[:, cols], av.at[i], sem_a.at[1, i]),
               pltpu.make_async_copy(aq_h.bitcast(U32).at[:, cols], aq.at[i], sem_a.at[2, i])]
        cps += [pltpu.make_async_copy(sk_h.bitcast(U32).at[pl.ds(i * 64, 64), pl.ds(m * C, C)], sk.at[i, m],
                                      sem_a.at[3, i]) for m in range(NC)]
        return cps

    x_copies = ([pltpu.make_async_copy(x_h.bitcast(U32).at[:, pl.ds(t * 128, 128)], x.at[t], sem_x.at[t])
                 for t in range(NT)] +
                [pltpu.make_async_copy(c_h.bitcast(U32).at[:, pl.ds(t * 128, 128)], c.at[t], sem_x.at[NT + t])
                 for t in range(NTC)])

    def w_copies(j, slot):
        cps = [pltpu.make_async_copy(w_h.bitcast(U32).at[:, j, :], dst.at[slot], sem_w.at[slot, n])
               for n, (w_h, dst) in enumerate([(wq_h, wq_raw), (wuk_h, wk_raw), (wuv_h, wv_raw)])]
        cps += [pltpu.make_async_copy(wo_h.bitcast(U32).at[j, :, pl.ds(t * 128, 128)], wo.at[slot, t],
                                      sem_w.at[slot, 3 + t]) for t in range(NT)]
        return cps

    for cp in w_copies(0, 0) + x_copies + a_copies(0):
        cp.start()

    sh = shift_ref[...].astype(F32)
    for i in range(NT):
        shift32[i, 0:4, :] = sh[:, i * 128:(i + 1) * 128]
        ak[i, 0:PAD, :] = jnp.zeros((PAD, 128), U32)
    d32[...] = ssmd_ref[...].astype(F32) * 0.5
    gate32[...] = gate_ref[...].astype(F32)
    for h in range(2):
        for n in range(3):
            dft[h, n] = pltpu.bitcast(dft_ref[h, n].astype(BF), U32)
    acc[...] = jnp.zeros(acc.shape, F32)
    zero_ref[...] = jnp.zeros((8, 128), U32)
    a_buf[...] = jnp.zeros(a_buf.shape, F32)
    for cp in x_copies:
        cp.wait()

    def unpack_pair(raw, slot, nt):
        lo, hi = [], []
        for t in range(nt):
            w = raw[slot, t * 128:(t + 1) * 128, :]
            lo.append(_lo(w).astype(BF))
            hi.append(_hi(w).astype(BF))
        return [lo, hi]

    def pair(j, carry):
        slot = j % 2
        ti = j // 2

        @pl.when(slot == 0)
        def _():
            for cp in a_copies(ti):
                cp.wait()

            @pl.when(ti + 1 < NT)
            def _():
                for cp in a_copies(ti + 1):
                    cp.start()

        for cp in w_copies(j, slot):
            cp.wait()

        @pl.when(j + 1 < NPAIR)
        def _():
            for cp in w_copies(j + 1, 1 - slot):
                cp.start()

        tri = (jax.lax.broadcasted_iota(jnp.int32, (128, 128), 1) <=
               jax.lax.broadcasted_iota(jnp.int32, (128, 128), 0))
        zero = zero_ref[...]

        def token(*vals):
            t = zero
            for v in vals:
                t = t & pltpu.bitcast(v, U32)
            return t

        def after(v, tok):
            head = pltpu.bitcast(pltpu.bitcast(v[0:8, :], U32) | tok, v.dtype)
            return head if v.shape[0] == 8 else jnp.concatenate([head, v[8:, :]], axis=0)

        def words(w, tok):
            return pltpu.bitcast(w if tok is None else after(w, tok), BF)

        qs, kk, vv, ctx, wts = {}, {}, {}, {}, {}

        ka, xs, kvs, kp, ys = {}, {}, {}, {}, {}
        HF = C // 2

        def fwd_k(m, tok):
            ka[m] = _mm_nt(words(dft[slot, 0], tok), pltpu.bitcast(sk[ti, m], BF))
            re, im = ka[m][0:HF, :], ka[m][HF:C, :]
            kp[m] = (im, -re) if m == 0 else (ka[m - 1][0:HF, :] + im, ka[m - 1][HF:C, :] - re)
            return ka[m]

        def fwd_x(cc, tok):
            r0 = PAD + cc * HF
            w0, w1, w2 = (ak[ti, r0 - d:r0 - d + HF, :] for d in range(3))
            s0, s1, s2, s3 = (jnp.broadcast_to(shift32[ti, d:d + 1, :], (8, 128)) for d in range(4))
            if KLAG:
                early = token(res[len(res) - KLAG][0:8, :])
                s0, s1, s2, s3 = (after(v, early) for v in (s0, s1, s2, s3))
            s0, s1, s2, s3 = (jnp.concatenate([v] * (HF // 8), axis=0) for v in (s0, s1, s2, s3))
            e0, o0, e1, o1, o2 = _lo(w0), _hi(w0), _lo(w1), _hi(w1), _hi(w2)
            wv = av[ti, cc * HF:(cc + 1) * HF, :]
            kv_e = (e0 * s0 + o1 * s1 + e1 * s2 + o2 * s3) * _lo(wv)
            kv_o = (o0 * s0 + e0 * s1 + o1 * s2 + e1 * s3) * _hi(wv)
            kvs[cc] = jnp.concatenate([kv_e, kv_o], axis=0)
            xs[cc] = _mm(words(dft[slot, 1], tok), kvs[cc].astype(BF))
            return xs[cc]

        def mac_steps():
            for r in range(HF // 8):
                rows = slice(r * 8, r * 8 + 8)
                for b in range(NC // MB):
                    ar, ai = [None] * MB, [None] * MB
                    for s_ in range(b * MB + MB):
                        gate = yield
                        xr, xi = xs[s_][rows, :], xs[s_][HF + r * 8:HF + r * 8 + 8, :]
                        if gate is not None:
                            xr, xi = after(xr, gate), after(xi, gate)
                        live = []
                        for u in range(MB):
                            m = b * MB + u - s_
                            if m < 0:
                                continue
                            kr, ki = kp[m][0][rows, :], kp[m][1][rows, :]
                            pr = xr * kr - xi * ki
                            pi = xr * ki + xi * kr
                            ar[u] = pr if ar[u] is None else ar[u] + pr
                            ai[u] = pi if ai[u] is None else ai[u] + pi
                            live += [ar[u], ai[u]]
                        if s_ == b * MB + MB - 1:
                            for u in range(MB):
                                ys[(b * MB + u, r)] = (ar[u], ai[u])
                        yield live

        def inv_y(cc, tok):
            yc = jnp.concatenate([ys[(cc, r)][0] for r in range(HF // 8)] +
                                 [ys[(cc, r)][1] for r in range(HF // 8)], axis=0)
            d = _mm(words(dft[slot, 2], tok), yc.astype(BF))
            y = d + kvs[cc] * d32[pl.ds(ti, 1), :]
            wq_ = aq[ti, cc * HF:(cc + 1) * HF, :]
            q = jnp.concatenate([_lo(wq_), _hi(wq_)], axis=0)
            a_buf[ti, cc * C:(cc + 1) * C, :] += q * y
            return d

        def proj_items(i, src, nt, name, dst, scale):
            items = []
            for e in range(2):
                st = {}

                def step(t, tok, e=e, st=st):
                    if name not in wts:
                        wts[name] = unpack_pair({"q": wq_raw, "k": wk_raw, "v": wv_raw}[name], slot, nt)
                    d = _mm(words(src[t, i * BQ // 2:(i + 1) * BQ // 2, :], tok), wts[name][e][t])
                    st["r"] = d if t == 0 else st["r"] + d
                    if t == nt - 1:
                        r = st["r"]
                        if scale is not None:
                            r = r * scale
                            for u in range(NSUB):
                                dst[(e, i, 128 * u)] = r[128 * u:, :].astype(BF)
                        else:
                            for u in range(NSUB):
                                dst[(e, i * NSUB + u)] = r[128 * u:128 * (u + 1), :].astype(BF)
                    return d
                items += [(True, P(step, t)) for t in range(nt)]
            return items

        def tiles(i):
            n0 = i * NSUB + 1
            return [(0, t) for t in range(n0)] + [(128 * w, n0 - 1 + w) for w in range(1, NSUB)]

        def qk_items(i, e, st):
            def step(ro, t, tok):
                s = _mm_nt(qs[(e, i, ro)], kk[(e, t)])
                for u in range(ro // 128, NSUB):
                    tl = s[128 * u - ro:128 * (u + 1) - ro, :]
                    if t == i * NSUB + u:
                        tl = jnp.where(tri, tl, NEG)
                    st["s"][(u, t)] = tl
                    st["mx"][u] = tl if st["mx"][u] is None else jnp.maximum(st["mx"][u], tl)
                    if t == i * NSUB + u:
                        st["m"][u] = jnp.max(st["mx"][u], axis=1, keepdims=True)
                return s
            return [(False, P(step, ro, t)) for ro, t in tiles(i)]

        def pv_items(i, e, st):
            def step(ro, t, last, tok):
                ps = []
                early = token(res[len(res) - XLAG][0:8, :]) if 2 * i + e >= XU else None
                for u in range(ro // 128, NSUB):
                    m = st["m"][u]
                    if early is not None:
                        m = jnp.broadcast_to(m, (128, 128))
                        m = jnp.concatenate([after(m[8 * n:8 * n + 8, :], early) for n in range(16)], axis=0)
                    p = jnp.exp2(st["s"].pop((u, t)) - m)
                    st["sm"][u] = p if st["sm"][u] is None else st["sm"][u] + p
                    ps.append(p)
                d = _mm(jnp.concatenate([p.astype(BF) for p in ps], axis=0), vv[(e, t)])
                for u in range(ro // 128, NSUB):
                    du = d[128 * u - ro:128 * (u + 1) - ro, :]
                    st["o"][u] = du if st["o"][u] is None else st["o"][u] + du
                if last:
                    parts = []
                    for u in range(NSUB):
                        l = jnp.broadcast_to(jnp.sum(st["sm"][u], axis=1, keepdims=True), (128, 128))
                        r = pl.reciprocal(l, approx=True)
                        r = r * (2.0 - l * r)
                        st["r"] += [r[8 * n:8 * n + 8, :] for n in range(16)]
                        parts.append(st["o"][u] * r)
                    ctx[(e, i)] = jnp.concatenate([v.astype(BF) for v in parts], axis=0)
                return d
            tl_ = tiles(i)
            return [(False, P(step, ro, t, n == len(tl_) - 1)) for n, (ro, t) in enumerate(tl_)]

        def out_items(i):
            st = {}

            def step(t, e, tok):
                d = _mm(ctx[(e, i)], words(wo[slot, t, e * HD // 2:(e + 1) * HD // 2, :], tok))
                if e == 0:
                    st["d"] = d
                else:
                    acc[t, i * BQ:(i + 1) * BQ, :] += st["d"] + d
                return d
            return [(True, P(step, t, e)) for t in range(NT) for e in range(2)]

        def new_state():
            return dict(s={}, mx=[None] * NSUB, m=[None] * NSUB, sm=[None] * NSUB, o=[None] * NSUB, r=[])

        P = functools.partial
        res = []
        units = [(i, e) for i in range(NB) for e in range(2)]
        states = [new_state() for _ in units]
        seq = [(True, P(fwd_k, m)) for m in range(NC)]
        seq += proj_items(0, x, NT, "q", qs, QSCALE) + proj_items(0, c, NTC, "k", kk, None)
        seq += qk_items(*units[0], states[0])
        seq += proj_items(0, c, NTC, "v", vv, None)
        marks = {}
        for n, (i, e) in enumerate(units):
            if n + 1 < len(units):
                seq += qk_items(*units[n + 1], states[n + 1])
            tail = []
            if e == 0:
                if i + 1 < NB:
                    fill = proj_items(i + 1, x, NT, "q", qs, QSCALE) + proj_items(i + 1, c, NTC, "k", kk, None)
                else:
                    fill = out_items(i - OD)
            else:
                fill = out_items(i - OD) if OD <= i < NB - 1 else []
                fill += proj_items(i + 1, c, NTC, "v", vv, None) if i + 1 < NB else []
                if i == 0:
                    fill += [(True, P(fwd_x, cc)) for cc in range(NC)]
                if i == NB - 1:
                    if OD == 2:
                        fill, tail = out_items(i - 1), [(True, P(inv_y, cc)) for cc in range(NC)]
                    else:
                        fill = [(True, P(inv_y, cc)) for cc in range(NC)]
            seq += _merge(fill, pv_items(i, e, states[n])) + tail
            marks[n] = len(seq)
        seq += out_items(NB - 1)

        mac = mac_steps()
        n_mac = (HF // 8) * sum(b * MB + MB for b in range(NC // MB))
        lo, hi = marks[MAC_LO], marks[MAC_HI]
        done_mac = 0
        prev_live = []
        deps = []
        for k, (gateable, item) in enumerate(seq):
            while k >= lo and done_mac < n_mac and done_mac * (hi - lo) < (k - lo + 1) * n_mac:
                next(mac)
                gate = token(res[k - MLAG][0:8, :]) if MLAG else None
                if E_MAC and prev_live:
                    gate = token(prev_live[-1]) if gate is None else gate & token(prev_live[-1])
                prev_live = mac.send(gate)
                if MDL:
                    deps += prev_live
                done_mac += 1
            if gateable and deps:
                res.append(item(token(*deps)))
                deps = []
            else:
                res.append(item(None))
        return carry
    jax.lax.fori_loop(0, NPAIR, pair, 0)

    cps = []
    HF = C // 2
    for cc in range(NC):
        gs = None
        for t in range(NT):
            w = aq[t, cc * HF:(cc + 1) * HF, :]
            term = jnp.concatenate([_lo(w), _hi(w)], axis=0) * gate32[t:t + 1, :]
            gs = term if gs is None else gs + term
        g = jax.nn.sigmoid(jnp.sum(gs, axis=1, keepdims=True))
        for t in range(NT):
            b = jnp.concatenate([acc[t, pl.ds(cc * C + par, HF, stride=2), :] for par in range(2)], axis=0)
            o = g * a_buf[t, cc * C:(cc + 1) * C, :] + (1.0 - g) * b
            out_v[cc * HF:(cc + 1) * HF, t * 128:(t + 1) * 128] = pltpu.pack_elementwise(
                [o[0:HF, :], o[HF:C, :]], packed_dtype=BF)
        cp = pltpu.make_async_copy(out_v.at[pl.ds(cc * HF, HF)], out_h.bitcast(U32).at[pl.ds(cc * HF, HF)],
                                   sem_o.at[cc])
        cp.start()
        cps.append(cp)
    for cp in cps:
        cp.wait()


@jax.jit
def pallas_gated_mix__ssm_conv_h3__compressed_kv_cla__prompt_kernel(
        A_q, A_k, A_v, A_shift_k, A_ssm_k, A_ssm_D, B_x, B_c_kv, B_w_q, B_w_uk, B_w_uv, B_w_o, gate_w):
    anyspec = pl.BlockSpec(memory_space=pl.ANY)
    vm = pl.BlockSpec(memory_space=pltpu.VMEM)
    V = pltpu.VMEM
    scratch = [
        V((NT, S // 2, 128), U32), V((NT, PAD + S // 2, 128), U32), V((NT, S // 2, 128), U32),
        V((NT, NC, 64, C), U32),
        V((NT, S // 2, 128), U32), V((NTC, S // 2, 128), U32),
        V((2, D, HD), U32), V((2, DC, HD), U32), V((2, DC, HD), U32), V((2, NT, HD, 128), U32),
        V((NT, S, 128), F32), V((NT, S, 128), F32), V((S // 2, D), U32),
        V((NT, 8, 128), F32), V((8, 128), F32), V((8, 128), F32), V((2, 3, C // 2, C), U32), V((8, 128), U32),
        pltpu.SemaphoreType.DMA((4, NT)), pltpu.SemaphoreType.DMA((NT + NTC,)),
        pltpu.SemaphoreType.DMA((2, 3 + NT)), pltpu.SemaphoreType.DMA((NC,)),
    ]
    out = pl.pallas_call(
        _kernel,
        out_shape=jax.ShapeDtypeStruct((S, D), BF),
        in_specs=[anyspec, anyspec, anyspec, vm, anyspec, vm, anyspec, anyspec, anyspec, anyspec, anyspec, anyspec,
                  vm, vm],
        out_specs=anyspec,
        scratch_shapes=scratch,
        compiler_params=pltpu.CompilerParams(vmem_limit_bytes=120 * 1024 * 1024, flags=_FLAGS),
    )(A_q.reshape(S, D), A_k.reshape(S, D), A_v.reshape(S, D), A_shift_k.T, A_ssm_k, A_ssm_D.reshape(NT, 128),
      B_x.reshape(S, D), B_c_kv.reshape(S, DC), B_w_q, B_w_uk, B_w_uv,
      B_w_o.reshape(NP, 2 * HD, D), gate_w.reshape(NT, 128), jnp.asarray(_DFT))
    return out.reshape(1, S, D)
```

```python
import functools
import os
import numpy as np
import jax
import jax.numpy as jnp
import jax.experimental.pallas as pl
import jax.experimental.pallas.tpu as pltpu

S, D, H, HD, DC, C = 2048, 1024, 32, 128, 512, 128
NC = S // C
NT = D // 128
NTC = DC // 128
NP = H // 2
BQ = 256
NB = S // BQ
NSUB = BQ // 128
HF = C // 2
HW = 64
PAD = 8
MB = 4
MAC_LO = int(os.environ.get("K_maclo", 3))
MAC_HI = int(os.environ.get("K_machi", 11))
MLAG = int(os.environ.get("K_mlag", 16))
KLAG = int(os.environ.get("K_klag", 14))
XLAG = int(os.environ.get("K_xlag", 8))
XU = int(os.environ.get("K_xu", 10))
E_MAC = int(os.environ.get("K_emac", 1))
P0 = int(os.environ.get("K_p0", 1))
FXS = int(os.environ.get("K_fxs", 2))
LOG2E = 1.4426950408889634
QSCALE = (HD ** -0.5) * LOG2E
NEG = -1e9 * LOG2E
BF = jnp.bfloat16
F32 = jnp.float32
U32 = jnp.uint32


def _dft_words():
    t_nat = np.arange(C, dtype=np.float64)
    t_par = np.concatenate([t_nat[0::2], t_nat[1::2]])
    mats = []
    for h in range(2):
        f = 2.0 * np.arange(h * HF, (h + 1) * HF, dtype=np.float64) + 0.5
        row = []
        for t in (t_nat, t_par):
            ang = 2.0 * np.pi * np.outer(f, t) / (2 * C)
            row.append(np.concatenate([np.cos(ang), -np.sin(ang)], axis=0))
        ang = 2.0 * np.pi * np.outer(t_par + C, f) / (2 * C)
        row.append(np.concatenate([np.cos(ang), -np.sin(ang)], axis=1) / C)
        mats.append(np.stack(row))
    bits = np.stack(mats).astype(np.float32).view(np.uint32)
    bits = (bits + np.uint32(0x7FFF) + ((bits >> np.uint32(16)) & np.uint32(1))) >> np.uint32(16)
    return (bits[:, :, 0::2, :] | (bits[:, :, 1::2, :] << np.uint32(16))).astype(np.uint32)


_DFT = _dft_words()


def _mm(a, b):
    return jnp.dot(a, b, preferred_element_type=F32)


def _mm_nt(a, b):
    return jax.lax.dot_general(a, b, (((1,), (1,)), ((), ())), preferred_element_type=F32)


def _bf(w):
    return pltpu.bitcast(w, BF)


def _lo(w):
    return pltpu.bitcast(w << 16, F32)


def _hi(w):
    return pltpu.bitcast(w & jnp.uint32(0xFFFF0000), F32)


def _lhs_terms(a11, a12, a21, a22):
    return [a11 + a22, a21 + a22, a11, a22, a11 + a12, a21 - a11, a12 - a22]


def _rhs_terms(b11, b12, b21, b22):
    return [b11 + b22, b11, b12 - b22, b21 - b11, b22, b11 + b12, b21 + b22]


def _combine(m):
    return m[0] + m[3] - m[4] + m[6], m[2] + m[4], m[1] + m[3], m[0] - m[1] + m[2] + m[5]


def _word_terms(terms, keep, *words):
    lo, hi = terms(*[_lo(w) for w in words]), terms(*[_hi(w) for w in words])
    return [words[keep[n]] if n in keep else pltpu.pack_elementwise([lo[n], hi[n]], packed_dtype=BF)
            for n in range(7)]


ORDER = [[0, 1, 2, 3, 4, 5, 6], [0, 3, 4, 6, 1, 2, 5], [6, 0, 3, 4, 2, 1, 5]][int(os.environ.get('K_ord', 1))]
LHS_KEEP = {2: 0, 3: 3}
RHS_KEEP = {1: 0, 4: 3}
LHS_SUMS = [n for n in range(7) if n not in LHS_KEEP]


def _merge(a, b):
    out, i, k = [], 0, 0
    while i < len(a) or k < len(b):
        if k >= len(b) or (i < len(a) and (i + 1) * len(b) <= (k + 1) * len(a)):
            out.append(a[i])
            i += 1
        else:
            out.append(b[k])
            k += 1
    return out


def _kernel(aq_h, ak_h, av_h, shift_h, sk_h, ssmd_h, x_h, c_h, wq_h, wuk_h, wuv_h, wo_h, gate_h, dft_h,
            out_h,
            aq, ak, av, sk, x, c, x_sums, c_sums, wq_raw, wk_raw, wv_raw, wo, a_part, a_buf, acc, out_v,
            shift_v, ssmd_v, gate_v, shift32, d32, gate32, dft, zero_ref,
            sem_a, sem_x, sem_w, sem_s, sem_o):
    P = functools.partial
    copy = pltpu.make_async_copy

    def a_copies(i):
        cols = pl.ds(i * 128, 128)
        return [copy(ak_h.bitcast(U32).at[:, cols], ak.at[i, pl.ds(PAD, S // 2)], sem_a.at[0, i]),
                copy(av_h.bitcast(U32).at[:, cols], av.at[i], sem_a.at[1, i]),
                copy(aq_h.bitcast(U32).at[:, cols], aq.at[i], sem_a.at[2, i]),
                copy(sk_h.bitcast(U32).at[pl.ds(i * 64, 64), :], sk.at[i], sem_a.at[3, i])]

    def x_copy(i):
        rows = pl.ds(i * BQ // 2, BQ // 2)
        return copy(x_h.bitcast(U32).at[rows], x.at[rows], sem_x.at[0, i])

    def c_copy(i):
        rows = pl.ds(i * BQ // 2, BQ // 2)
        return copy(c_h.bitcast(U32).at[rows], c.at[rows], sem_x.at[1, i])

    def w_copies(j, slot):
        cps = [copy(w_h.bitcast(U32).at[:, j, :], dst.at[slot], sem_w.at[slot, n])
               for n, (w_h, dst) in enumerate([(wq_h, wq_raw), (wuk_h, wk_raw), (wuv_h, wv_raw)])]
        return cps + [copy(wo_h.bitcast(U32).at[j], wo.at[slot], sem_w.at[slot, 3])]

    small = [copy(s_, d_, sem_s.at[n]) for n, (s_, d_) in enumerate(
        [(shift_h, shift_v), (ssmd_h, ssmd_v), (gate_h, gate_v), (dft_h, dft)])]

    def body(j):
        slot = j & 1
        zero = zero_ref[...]
        tri = (jax.lax.broadcasted_iota(jnp.int32, (128, 128), 1) <=
               jax.lax.broadcasted_iota(jnp.int32, (128, 128), 0))
        res = []

        def token(lag):
            return zero & pltpu.bitcast(res[max(len(res) - lag, 0)][0:8, :], U32)

        def after(v, tok):
            return pltpu.bitcast(pltpu.bitcast(v, U32) | tok, F32)

        def ssm_part(ti, fh):
            ka, xs, kvs, ys = {}, {}, {}, {}

            def fwd_k(m):
                ka[m] = _mm_nt(_bf(dft[fh, 0]), _bf(sk[ti, :, m * C:(m + 1) * C]))
                return ka[m]

            def fwd_x(cc):
                r0 = PAD + cc * HF
                w0, w1, w2 = (ak[ti, r0 - d:r0 - d + HF, :] for d in range(3))
                early = token(KLAG)
                s0, s1, s2, s3 = (
                    jnp.concatenate([after(jnp.broadcast_to(shift32[ti, d:d + 1, :], (8, 128)), early)] * (HF // 8),
                                    axis=0) for d in range(4))
                e0, o0, e1, o1, o2 = _lo(w0), _hi(w0), _lo(w1), _hi(w1), _hi(w2)
                wv = av[ti, cc * HF:(cc + 1) * HF, :]
                kv_e = (e0 * s0 + o1 * s1 + e1 * s2 + o2 * s3) * _lo(wv)
                kv_o = (o0 * s0 + e0 * s1 + o1 * s2 + e1 * s3) * _hi(wv)
                kvs[cc] = jnp.concatenate([kv_e, kv_o], axis=0)
                xs[cc] = _mm(_bf(dft[fh, 1]), kvs[cc].astype(BF))
                return xs[cc]

            def mac_steps():
                for r in range(HF // 8):
                    rows = slice(r * 8, r * 8 + 8)
                    for b in range(NC // MB):
                        ar, ai = [None] * MB, [None] * MB
                        for s_ in range(b * MB + MB):
                            gate = yield
                            xr = after(xs[s_][rows, :], gate)
                            xi = after(xs[s_][HF + r * 8:HF + r * 8 + 8, :], gate)
                            for u in range(MB):
                                m = b * MB + u - s_
                                if m < 0:
                                    continue
                                kr, ki = ka[m][rows, :], ka[m][HF + r * 8:HF + r * 8 + 8, :]
                                pr = xr * kr - xi * ki
                                pi = xr * ki + xi * kr
                                ar[u] = pr if ar[u] is None else ar[u] + pr
                                ai[u] = pi if ai[u] is None else ai[u] + pi
                            if s_ == b * MB + MB - 1:
                                for u in range(MB):
                                    ys[(b * MB + u, r)] = (ar[u], ai[u])
                            yield ai[MB - 1]

            def inv_y(cc):
                if cc == 0:
                    re = [ys[(0, r)][1] for r in range(HF // 8)]
                    im = [-ys[(0, r)][0] for r in range(HF // 8)]
                else:
                    re = [ys[(cc - 1, r)][0] + ys[(cc, r)][1] for r in range(HF // 8)]
                    im = [ys[(cc - 1, r)][1] - ys[(cc, r)][0] for r in range(HF // 8)]
                yc = jnp.concatenate(re + im, axis=0)
                d = _mm(_bf(dft[fh, 2]), yc.astype(BF))
                y = d + kvs[cc] * d32[pl.ds(ti, 1), :]
                wq_ = aq[ti, cc * HF:(cc + 1) * HF, :]
                a = jnp.concatenate([_lo(wq_), _hi(wq_)], axis=0) * y
                rows = slice(cc * C, (cc + 1) * C)
                if isinstance(fh, int):
                    a = a + a_part[rows, :] if fh else a
                else:
                    a = a + jnp.where(fh == 1, a_part[rows, :], 0.0)
                a_part[rows, :] = a
                a_buf[cc * HF:(cc + 1) * HF, pl.ds(pl.multiple_of(ti * 128, 128), 128)] = pltpu.pack_elementwise(
                    [a[0:HF, :], a[HF:C, :]], packed_dtype=BF)
                return d

            return ([P(fwd_k, m) for m in range(NC)], [P(fwd_x, cc) for cc in range(NC)], mac_steps(),
                    [P(inv_y, cc) for cc in range(NC)])

        qs, kk, vv, ctx, wts, gates = {}, {}, {}, {}, {}, {}

        def proj_items(i, name):
            src, sums, nt, raw, dst = {"q": (x, x_sums, NT // 2, wq_raw, qs), "k": (c, c_sums, NTC // 2, wk_raw, kk),
                                       "v": (c, c_sums, NTC // 2, wv_raw, vv)}[name]
            m = [None] * 7

            def step(n, t):
                if (name, t) not in wts:
                    top = raw[slot, t * 128:(t + 1) * 128, :]
                    bot = raw[slot, (t + nt) * 128:(t + nt + 1) * 128, :]
                    wts[(name, t)] = [v.astype(BF) for v in _rhs_terms(_lo(top), _hi(top), _lo(bot), _hi(bot))]
                if n in LHS_KEEP:
                    h = LHS_KEEP[n] // 3
                    lhs = src[(2 * i + h) * HW:(2 * i + h + 1) * HW, (t + h * nt) * 128:(t + h * nt + 1) * 128]
                else:
                    lhs = sums[LHS_SUMS.index(n), i * HW:(i + 1) * HW, t * 128:(t + 1) * 128]
                d = _mm(_bf(lhs), wts[(name, t)][n])
                m[n] = d if t == 0 else m[n] + d
                if n == ORDER[-1] and t == nt - 1:
                    c11, c12, c21, c22 = _combine(m)
                    for e, (top, bot) in enumerate([(c11, c21), (c12, c22)]):
                        if name == "q":
                            top, bot = (top * QSCALE).astype(BF), (bot * QSCALE).astype(BF)
                            dst[(e, i, 0)] = jnp.concatenate([top, bot], axis=0)
                            dst[(e, i, 128)] = bot
                        else:
                            dst[(e, i * NSUB)] = top.astype(BF)
                            dst[(e, i * NSUB + 1)] = bot.astype(BF)
                return d
            return [P(step, n, t) for n in ORDER for t in range(nt)]

        def tiles(i):
            n0 = i * NSUB + 1
            return [(0, t) for t in range(n0)] + [(128 * w, n0 - 1 + w) for w in range(1, NSUB)]

        def qk_items(i, e, st):
            def step(ro, t):
                s = _mm_nt(qs[(e, i, ro)], kk[(e, t)])
                for u in range(ro // 128, NSUB):
                    tl = s[128 * u - ro:128 * (u + 1) - ro, :]
                    if t == i * NSUB + u:
                        tl = jnp.where(tri, tl, NEG)
                    st["s"][(u, t)] = tl
                    st["mx"][u] = tl if t == 0 else jnp.maximum(st["mx"][u], tl)
                    if t == i * NSUB + u:
                        st["m"][u] = jnp.max(st["mx"][u], axis=1, keepdims=True)
                return s
            return [P(step, ro, t) for ro, t in tiles(i)]

        def pv_items(i, e, st):
            def step(ro, t):
                ps = []
                early = token(XLAG) if 2 * i + e >= XU else None
                for u in range(ro // 128, NSUB):
                    m = st["m"][u]
                    if early is not None:
                        m = jnp.broadcast_to(m, (128, 128))
                        m = jnp.concatenate([after(m[8 * n:8 * n + 8, :], early) for n in range(16)], axis=0)
                    p = jnp.exp2(st["s"].pop((u, t)) - m)
                    st["sm"][u] = p if t == 0 else st["sm"][u] + p
                    ps.append(p.astype(BF))
                d = _mm(jnp.concatenate(ps, axis=0), vv[(e, t)])
                for u in range(ro // 128, NSUB):
                    du = d[128 * u - ro:128 * (u + 1) - ro, :]
                    st["o"][u] = du if t == 0 else st["o"][u] + du
                if t == (i + 1) * NSUB - 1:
                    for u in range(NSUB):
                        l = jnp.sum(st["sm"][u], axis=1, keepdims=True)
                        r = pl.reciprocal(l, approx=True)
                        r = r * (2.0 - l * r)
                        ctx[(e, i, u)] = st["o"][u] * r
                return d
            return [P(step, ro, t) for ro, t in tiles(i)]

        def out_items(i):
            st = {}
            m = [None] * 7
            nt = NT // 2

            def step(t, n):
                left, right = slice(t * 128, (t + 1) * 128), slice((t + nt) * 128, (t + nt + 1) * 128)
                if ("o", t) not in wts:
                    wts[("o", t)] = _word_terms(_rhs_terms, RHS_KEEP, wo[slot, 0:HW, left], wo[slot, 0:HW, right],
                                                wo[slot, HW:2 * HW, left], wo[slot, HW:2 * HW, right])
                if not st:
                    st["lhs"] = [v.astype(BF) for v in _lhs_terms(
                        ctx[(0, i, 0)], ctx[(1, i, 0)], ctx[(0, i, 1)], ctx[(1, i, 1)])]
                m[n] = _mm(st["lhs"][n], _bf(wts[("o", t)][n]))
                if n == ORDER[-1]:
                    top, bot = slice(i * BQ, i * BQ + 128), slice(i * BQ + 128, (i + 1) * BQ)
                    for (rows, cols), v in zip([(top, left), (top, right), (bot, left), (bot, right)], _combine(m)):
                        acc[rows, cols] += v
                return m[n]
            return [P(step, t, n) for t in range(nt) for n in ORDER]

        units = [(i, e) for i in range(NB) for e in range(2)]
        states = [dict(s={}, mx=[None] * NSUB, m=[None] * NSUB, sm=[None] * NSUB, o=[None] * NSUB) for _ in units]
        head, extra, tail, macs = [], {}, [], []
        fk, fx, mac, inv = ssm_part(j >> 1, j & 1)
        tail = inv
        head = fk
        for n in range(FXS):
            extra[MAC_LO - FXS + 1 + n] = fx[n * NC // FXS:(n + 1) * NC // FXS]
        macs.append((mac, MAC_LO, MAC_HI))

        if P0 == 0:
            seq = head + proj_items(0, "q") + proj_items(0, "k") + qk_items(*units[0], states[0]) + proj_items(0, "v")
        elif P0 == 1:
            seq = head + proj_items(0, "k") + proj_items(0, "q") + proj_items(0, "v") + qk_items(*units[0], states[0])
        elif P0 == 2:
            seq = (head[:8] + _merge(head[8:], proj_items(0, "k")) + proj_items(0, "q") + proj_items(0, "v") +
                   qk_items(*units[0], states[0]))
        elif P0 == 3:
            seq = (head[:8] + _merge(head[8:], proj_items(0, "k") + proj_items(0, "v")) + proj_items(0, "q") +
                   qk_items(*units[0], states[0]))
        marks = {}
        for n, (i, e) in enumerate(units):
            if n + 1 < len(units):
                seq += qk_items(*units[n + 1], states[n + 1])
            if i + 1 == NB:
                fill = out_items(i - 2 + e)
            elif e == 0:
                fill = proj_items(i + 1, "q") + proj_items(i + 1, "k")
            else:
                fill = (out_items(i - 2) if i >= 2 else []) + proj_items(i + 1, "v")
            seq += _merge(_merge(fill, extra.get(n, [])), pv_items(i, e, states[n]))
            marks[n] = len(seq)
        seq += tail + out_items(NB - 1)

        n_mac = (HF // 8) * sum(b * MB + MB for b in range(NC // MB))
        done = [0] * len(macs)
        prev = None
        for k, item in enumerate(seq):
            for n, (mac, s0, s1) in enumerate(macs):
                lo, hi = marks[s0], marks[s1]
                while k >= lo and done[n] < n_mac and done[n] * (hi - lo) < (k - lo + 1) * n_mac:
                    next(mac)
                    gate = token(MLAG)
                    if E_MAC and prev is not None:
                        gate = gate & pltpu.bitcast(prev, U32)
                    prev = mac.send(gate)
                    done[n] += 1
            res.append(item())

    out_copies = {hi - 1: copy(out_v.at[pl.ds(lo * BQ, (hi - lo) * BQ)], out_h.at[pl.ds(lo * BQ, (hi - lo) * BQ)],
                               sem_o.at[n])
                  for n, (lo, hi) in enumerate([(i, i + 1) for i in range(NB)])}

    first = w_copies(0, 0) + small + a_copies(0)
    for cp in [cp for i in range(NB) for cp in (x_copy(i), c_copy(i))] + first:
        cp.start()
    zero_ref[...] = jnp.zeros((8, 128), U32)
    for t in range(NT):
        ak[t, 0:PAD, :] = jnp.zeros((PAD, 128), U32)
    acc[...] = jnp.zeros(acc.shape, F32)
    for i in range(NB):
        for cp, src, sums, half in ((x_copy(i), x, x_sums, D // 2), (c_copy(i), c, c_sums, DC // 2)):
            cp.wait()
            top, bot = slice(2 * i * HW, (2 * i + 1) * HW), slice((2 * i + 1) * HW, (2 * i + 2) * HW)
            terms = _word_terms(_lhs_terms, LHS_KEEP, src[top, 0:half], src[top, half:], src[bot, 0:half],
                                src[bot, half:])
            for k, n in enumerate(LHS_SUMS):
                sums[k, i * HW:(i + 1) * HW, :] = terms[n]
    for cp in first:
        cp.wait()
    sh = shift_v[...].astype(F32)
    for t in range(NT):
        shift32[t, 0:4, :] = sh[:, t * 128:(t + 1) * 128]
    d32[...] = ssmd_v[...].astype(F32) * 0.5
    gate32[...] = gate_v[...].astype(F32)

    def middle(j, carry):
        ti = j >> 1

        @pl.when(j > 0)
        def _():
            @pl.when((j & 1) == 0)
            def _():
                for cp in a_copies(ti):
                    cp.wait()
            for cp in w_copies(j, j & 1):
                cp.wait()

        @pl.when(j + 1 < NP)
        def _():
            for cp in w_copies(j + 1, 1 - (j & 1)):
                cp.start()

            @pl.when((j & 1) == 1)
            def _():
                for cp in a_copies(ti + 1):
                    cp.start()
        body(j)
        return carry
    jax.lax.fori_loop(0, NP, middle, 0)

    for i in range(NB):
        rows = slice(i * BQ, (i + 1) * BQ)
        wrows = slice(i * BQ // 2, (i + 1) * BQ // 2)
        gs = None
        for n in range(NT):
            term = _bf(aq[n, wrows, :]).astype(F32) * gate32[n:n + 1, :]
            gs = term if gs is None else gs + term
        g = jax.nn.sigmoid(jnp.sum(gs, axis=1, keepdims=True))
        for t in range(NT):
            cols = slice(t * 128, (t + 1) * 128)
            out_v[rows, cols] = (g * _bf(a_buf[wrows, cols]).astype(F32) + (1.0 - g) * acc[rows, cols]).astype(BF)
        out_copies[i].start()
    for cp in out_copies.values():
        cp.wait()


@jax.jit
def pallas_gated_mix__ssm_conv_h3__compressed_kv_cla__prompt_kernel(
        A_q, A_k, A_v, A_shift_k, A_ssm_k, A_ssm_D, B_x, B_c_kv, B_w_q, B_w_uk, B_w_uv, B_w_o, gate_w):
    V = pltpu.VMEM
    dma = pltpu.SemaphoreType.DMA
    scratch = [
        V((NT, S // 2, 128), U32), V((NT, PAD + S // 2, 128), U32), V((NT, S // 2, 128), U32), V((NT, 64, S), U32),
        V((S // 2, D), U32), V((S // 2, DC), U32), V((5, NB * HW, D // 2), U32), V((5, NB * HW, DC // 2), U32),
        V((2, D, HD), U32), V((2, DC, HD), U32), V((2, DC, HD), U32), V((2, HD, D), U32),
        V((S, 128), F32), V((S // 2, D), U32), V((S, D), F32), V((S, D), BF),
        V((4, D), BF), V((NT, 128), BF), V((NT, 128), BF),
        V((NT, 8, 128), F32), V((NT, 128), F32), V((NT, 128), F32), V((2, 3, HF, C), U32), V((8, 128), U32),
        dma((4, NT)), dma((2, NB)), dma((2, 4)), dma((4,)), dma((NB,)),
    ]
    out = pl.pallas_call(
        _kernel,
        out_shape=jax.ShapeDtypeStruct((S, D), BF),
        in_specs=[pl.BlockSpec(memory_space=pl.ANY)] * 14,
        out_specs=pl.BlockSpec(memory_space=pl.ANY),
        scratch_shapes=scratch,
        compiler_params=pltpu.CompilerParams(vmem_limit_bytes=120 * 1024 * 1024, disable_bounds_checks=True),
    )(A_q.reshape(S, D), A_k.reshape(S, D), A_v.reshape(S, D), A_shift_k.T, A_ssm_k, A_ssm_D.reshape(NT, 128),
      B_x.reshape(S, D), B_c_kv.reshape(S, DC), B_w_q, B_w_uk, B_w_uv,
      B_w_o.reshape(NP, 2 * HD, D), gate_w.reshape(NT, 128), jnp.asarray(_DFT))
    return out.reshape(1, S, D)
```

```python
import functools
import os

import numpy as np
import jax
import jax.numpy as jnp
import jax.experimental.pallas as pl
import jax.experimental.pallas.tpu as pltpu

S, D, H, HD, DC = 2048, 1024, 32, 128, 512
NT, NTC = D // 128, DC // 128
NP = H // 2
BQ = 256
NB = S // BQ
HW = 64
C = 128
NC = S // C
HF = C // 2
MB = 4
PAD = 8

FWD_AT = int(os.environ.get("K_fwd", 1))
FXS = int(os.environ.get("K_fxs", 3))
MAC_END = int(os.environ.get("K_machi", 9))
INV_AT = int(os.environ.get("K_inv", 11))
PACED_FROM = int(os.environ.get("K_xu", 9))
MAC_LAG = int(os.environ.get("K_mlag", 24))
KV_LAG = int(os.environ.get("K_klag", 14))
EXP_LAG = int(os.environ.get("K_xlag", 11))
ORDER = [[0, 1, 2, 3, 4, 5, 6], [0, 3, 4, 6, 1, 2, 5], [6, 0, 3, 4, 2, 1, 5]][int(os.environ.get('K_ord', 2))]

LOG2E = 1.4426950408889634
QSCALE = (HD ** -0.5) * LOG2E
MASKED = -1e9 * LOG2E
BF, F32, U32 = jnp.bfloat16, jnp.float32, jnp.uint32


def _dft_words():
    t_nat = np.arange(C, dtype=np.float64)
    t_par = np.concatenate([t_nat[0::2], t_nat[1::2]])
    mats = []
    for h in range(2):
        f = 2.0 * np.arange(h * HF, (h + 1) * HF, dtype=np.float64) + 0.5
        row = []
        for t in (t_nat, t_par):
            ang = 2.0 * np.pi * np.outer(f, t) / (2 * C)
            row.append(np.concatenate([np.cos(ang), -np.sin(ang)], axis=0))
        ang = 2.0 * np.pi * np.outer(t_par + C, f) / (2 * C)
        row.append(np.concatenate([np.cos(ang), -np.sin(ang)], axis=1) / C)
        mats.append(np.stack(row))
    bits = np.stack(mats).astype(np.float32).view(np.uint32)
    bits = (bits + np.uint32(0x7FFF) + ((bits >> np.uint32(16)) & np.uint32(1))) >> np.uint32(16)
    return (bits[:, :, 0::2, :] | (bits[:, :, 1::2, :] << np.uint32(16))).astype(np.uint32)


_DFT = _dft_words()


def _mm(a, b):
    return jnp.dot(a, b, preferred_element_type=F32)


def _mm_nt(a, b):
    return jax.lax.dot_general(a, b, (((1,), (1,)), ((), ())), preferred_element_type=F32)


def _bf(words):
    return pltpu.bitcast(words, BF)


def _lo(words):
    return pltpu.bitcast(words << 16, F32)


def _hi(words):
    return pltpu.bitcast(words & jnp.uint32(0xFFFF0000), F32)


def _pack(even_rows, odd_rows):
    return pltpu.pack_elementwise([even_rows, odd_rows], packed_dtype=BF)


def _lhs_terms(a11, a12, a21, a22):
    return [a11 + a22, a21 + a22, a11, a22, a11 + a12, a21 - a11, a12 - a22]


def _rhs_terms(b11, b12, b21, b22):
    return [b11 + b22, b11, b12 - b22, b21 - b11, b22, b11 + b12, b21 + b22]


def _combine(m):
    return m[0] + m[3] - m[4] + m[6], m[2] + m[4], m[1] + m[3], m[0] - m[1] + m[2] + m[5]


LHS_PLAIN = {2: 0, 3: 3}
RHS_PLAIN = {1: 0, 4: 3}
LHS_SUMS = [n for n in range(7) if n not in LHS_PLAIN]


def _word_terms(terms, plain, *words):
    lo, hi = terms(*[_lo(w) for w in words]), terms(*[_hi(w) for w in words])
    return [words[plain[n]] if n in plain else _pack(lo[n], hi[n]) for n in range(7)]


def _merge(a, b):
    out, i, k = [], 0, 0
    while i < len(a) or k < len(b):
        if k >= len(b) or (i < len(a) and (i + 1) * len(b) <= (k + 1) * len(a)):
            out.append(a[i])
            i += 1
        else:
            out.append(b[k])
            k += 1
    return out


def _tile(n):
    return slice(n * 128, (n + 1) * 128)


def _half(n):
    return slice(n * HW, (n + 1) * HW)


def _kernel(aq_h, ak_h, av_h, shift_h, sk_h, ssmd_h, x_h, c_h, wq_h, wuk_h, wuv_h, wo_h, gate_h, dft_h, out_h,
            aq, ak, av, sk, x, c, x_sums, c_sums, wq, wk, wv, wo, y_half, y_buf, acc, out_v,
            shift_v, ssmd_v, gate_v, shift32, ssmd32, dft, zero_ref,
            sem_a, sem_x, sem_w, sem_s, sem_o):
    P = functools.partial
    copy = pltpu.make_async_copy

    def ssm_copies(i):
        cols = pl.ds(i * 128, 128)
        return [copy(ak_h.bitcast(U32).at[:, cols], ak.at[i, pl.ds(PAD, S // 2)], sem_a.at[0, i]),
                copy(av_h.bitcast(U32).at[:, cols], av.at[i], sem_a.at[1, i]),
                copy(sk_h.bitcast(U32).at[pl.ds(i * HW, HW), :], sk.at[i], sem_a.at[2, i])]

    def row_copy(src, dst, n, i):
        rows = pl.ds(i * BQ // 2, BQ // 2)
        return copy(src.bitcast(U32).at[rows], dst.at[rows], sem_x.at[n, i])

    def weight_copies(j):
        slot = j & 1
        cps = [copy(src.bitcast(U32).at[:, j, :], dst.at[slot], sem_w.at[slot, n])
               for n, (src, dst) in enumerate([(wq_h, wq), (wuk_h, wk), (wuv_h, wv)])]
        return cps + [copy(wo_h.bitcast(U32).at[j], wo.at[slot], sem_w.at[slot, 3])]

    aq_copy = copy(aq_h.bitcast(U32), aq, sem_s.at[4])

    def head_pair(j):
        slot = j & 1
        ti = j >> 1
        zero = zero_ref[...]
        causal = (jax.lax.broadcasted_iota(jnp.int32, (128, 128), 1) <=
                  jax.lax.broadcasted_iota(jnp.int32, (128, 128), 0))
        issued = []

        def token(lag):
            return zero & pltpu.bitcast(issued[max(len(issued) - lag, 0)][0:8, :], U32)

        def after(v, tok):
            return pltpu.bitcast(pltpu.bitcast(v, U32) | tok, F32)

        k_spec, x_spec, kv, y_spec = {}, {}, {}, {}

        def transform_filter(m):
            k_spec[m] = _mm_nt(_bf(dft[slot, 0]), _bf(sk[ti, :, _tile(m)]))
            return k_spec[m]

        def transform_input(n):
            r0 = PAD + n * HW
            w0, w1, w2 = (ak[ti, r0 - d:r0 - d + HW, :] for d in range(3))
            tok = token(KV_LAG)
            s0, s1, s2, s3 = (
                jnp.concatenate([after(jnp.broadcast_to(shift32[ti, d:d + 1, :], (8, 128)), tok)] * (HW // 8), axis=0)
                for d in range(4))
            e0, o0, e1, o1, o2 = _lo(w0), _hi(w0), _lo(w1), _hi(w1), _hi(w2)
            v = av[ti, _half(n), :]
            kv[n] = jnp.concatenate([(e0 * s0 + o1 * s1 + e1 * s2 + o2 * s3) * _lo(v),
                                     (o0 * s0 + e0 * s1 + o1 * s2 + e1 * s3) * _hi(v)], axis=0)
            x_spec[n] = _mm(_bf(dft[slot, 1]), kv[n].astype(BF))
            return x_spec[n]

        def spectral_product():
            for r in range(HF // 8):
                re, im = slice(r * 8, r * 8 + 8), slice(HF + r * 8, HF + r * 8 + 8)
                for b in range(NC // MB):
                    acc_re, acc_im = [None] * MB, [None] * MB
                    for n in range((b + 1) * MB):
                        tok = yield
                        xr, xi = after(x_spec[n][re, :], tok), after(x_spec[n][im, :], tok)
                        for u in range(MB):
                            m = b * MB + u - n
                            if m >= 0:
                                kr, ki = k_spec[m][re, :], k_spec[m][im, :]
                                pr, pi = xr * kr - xi * ki, xr * ki + xi * kr
                                acc_re[u] = pr if n == 0 else acc_re[u] + pr
                                acc_im[u] = pi if n == 0 else acc_im[u] + pi
                                y_spec[(b * MB + u, r)] = (acc_re[u], acc_im[u])
                        yield acc_im[MB - 1]

        def transform_back(n):
            cur = [y_spec[(n, r)] for r in range(HF // 8)]
            if n == 0:
                parts = [im for _, im in cur] + [-re for re, _ in cur]
            else:
                old = [y_spec[(n - 1, r)] for r in range(HF // 8)]
                parts = [o[0] + v[1] for o, v in zip(old, cur)] + [o[1] - v[0] for o, v in zip(old, cur)]
            conv = _mm(_bf(dft[slot, 2]), jnp.concatenate(parts, axis=0).astype(BF))
            y = conv + kv[n] * ssmd32[pl.ds(ti, 1), :] + jnp.where(slot == 1, y_half[_tile(n), :], 0.0)
            y_half[_tile(n), :] = y
            y_buf[_half(n), pl.ds(pl.multiple_of(ti * 128, 128), 128)] = _pack(y[0:HW, :], y[HW:, :])
            return conv

        qs, ks, vs, ctx, rhs = {}, {}, {}, {}, {}

        def project(i, name):
            src, sums, nt, w = {"q": (x, x_sums, NT // 2, wq), "k": (c, c_sums, NTC // 2, wk),
                                "v": (c, c_sums, NTC // 2, wv)}[name]
            m = [None] * 7

            def step(n, t):
                if (name, t) not in rhs:
                    top, bot = w[slot, _tile(t), :], w[slot, _tile(t + nt), :]
                    rhs[(name, t)] = [v.astype(BF) for v in _rhs_terms(_lo(top), _hi(top), _lo(bot), _hi(bot))]
                if n in LHS_PLAIN:
                    h = LHS_PLAIN[n] // 3
                    lhs = src[_half(2 * i + h), _tile(t + h * nt)]
                else:
                    lhs = sums[LHS_SUMS.index(n), _half(i), _tile(t)]
                d = _mm(_bf(lhs), rhs[(name, t)][n])
                m[n] = d if t == 0 else m[n] + d
                if n == ORDER[-1] and t == nt - 1:
                    c11, c12, c21, c22 = _combine(m)
                    for e, (top, bot) in enumerate([(c11, c21), (c12, c22)]):
                        if name == "q":
                            top, bot = (top * QSCALE).astype(BF), (bot * QSCALE).astype(BF)
                            qs[(e, i, 0)] = jnp.concatenate([top, bot], axis=0)
                            qs[(e, i, 1)] = bot
                        else:
                            dst = ks if name == "k" else vs
                            dst[(e, 2 * i)], dst[(e, 2 * i + 1)] = top.astype(BF), bot.astype(BF)
                return d
            return [P(step, n, t) for n in ORDER for t in range(nt)]

        def key_tiles(i):
            return [(0, t) for t in range(2 * i + 1)] + [(1, 2 * i + 1)]

        def scores(i, e, st):
            def step(u0, t):
                s = _mm_nt(qs[(e, i, u0)], ks[(e, t)])
                for u in range(u0, 2):
                    part = s[_tile(u - u0), :]
                    if t == 2 * i + u:
                        part = jnp.where(causal, part, MASKED)
                    st["s"][(u, t)] = part
                    st["max"][u] = part if t == 0 else jnp.maximum(st["max"][u], part)
                    if t == 2 * i + u:
                        st["max"][u] = jnp.max(st["max"][u], axis=1, keepdims=True)
                return s
            return [P(step, u0, t) for u0, t in key_tiles(i)]

        def attend(i, e, st):
            def step(u0, t):
                tok = token(EXP_LAG) if 2 * i + e >= PACED_FROM else None
                probs = []
                for u in range(u0, 2):
                    m = st["max"][u]
                    if tok is not None:
                        m = jnp.broadcast_to(m, (128, 128))
                        m = jnp.concatenate([after(m[8 * n:8 * n + 8, :], tok) for n in range(16)], axis=0)
                    p = jnp.exp2(st["s"].pop((u, t)) - m)
                    st["sum"][u] = p if t == 0 else st["sum"][u] + p
                    probs.append(p.astype(BF))
                d = _mm(jnp.concatenate(probs, axis=0), vs[(e, t)])
                for u in range(u0, 2):
                    part = d[_tile(u - u0), :]
                    st["out"][u] = part if t == 0 else st["out"][u] + part
                if u0 == 1:
                    for u in range(2):
                        total = jnp.sum(st["sum"][u], axis=1, keepdims=True)
                        r = pl.reciprocal(total, approx=True)
                        ctx[(e, i, u)] = st["out"][u] * (r * (2.0 - total * r))
                return d
            return [P(step, u0, t) for u0, t in key_tiles(i)]

        def project_out(i):
            lhs, m = [], [None] * 7

            def step(t, n):
                left, right = _tile(t), _tile(t + NT // 2)
                if ("o", t) not in rhs:
                    rhs[("o", t)] = _word_terms(_rhs_terms, RHS_PLAIN, *[
                        wo[slot, _half(e), cols] for e in range(2) for cols in (left, right)])
                if not lhs:
                    lhs.extend(v.astype(BF) for v in _lhs_terms(
                        ctx[(0, i, 0)], ctx[(1, i, 0)], ctx[(0, i, 1)], ctx[(1, i, 1)]))
                m[n] = _mm(lhs[n], _bf(rhs[("o", t)][n]))
                if n == ORDER[-1]:
                    blocks = [(_tile(2 * i + u), cols) for u in range(2) for cols in (left, right)]
                    for block, v in zip(blocks, _combine(m)):
                        acc[block] += v
                return m[n]
            return [P(step, t, n) for t in range(NT // 2) for n in ORDER]

        units = [(i, e) for i in range(NB) for e in range(2)]
        states = [dict(s={}, max=[None] * 2, sum=[None] * 2, out=[None] * 2) for _ in units]
        extra = {FWD_AT + n: [P(transform_input, k) for k in range(n * NC // FXS, (n + 1) * NC // FXS)]
                 for n in range(FXS)}
        extra[INV_AT] = [P(transform_back, n) for n in range(NC)]
        seq = [P(transform_filter, m) for m in range(NC)]
        seq += project(0, "k") + project(0, "q") + project(0, "v") + scores(*units[0], states[0])
        ends = []
        for n, (i, e) in enumerate(units):
            if n + 1 < len(units):
                seq += scores(*units[n + 1], states[n + 1])
            if i + 1 == NB:
                fill = project_out(i - 2 + e)
            elif e == 0:
                fill = project(i + 1, "q") + project(i + 1, "k")
            else:
                fill = (project_out(i - 2) if i >= 2 else []) + project(i + 1, "v")
            seq += _merge(_merge(fill, extra.get(n, [])), attend(i, e, states[n]))
            ends.append(len(seq))
        seq += project_out(NB - 1)

        product = spectral_product()
        steps = (HF // 8) * sum((b + 1) * MB for b in range(NC // MB))
        lo, hi = ends[FWD_AT + FXS - 1], ends[MAC_END]
        done, last = 0, None
        for k, item in enumerate(seq):
            while k >= lo and done < steps and done * (hi - lo) < (k - lo + 1) * steps:
                next(product)
                tok = token(MAC_LAG)
                last = product.send(tok if last is None else tok & pltpu.bitcast(last, U32))
                done += 1
            issued.append(item())

    first = weight_copies(0) + ssm_copies(0) + [
        copy(src, dst, sem_s.at[n]) for n, (src, dst) in enumerate(
            [(shift_h, shift_v), (ssmd_h, ssmd_v), (gate_h, gate_v), (dft_h, dft)])]
    rows_in = [(i, row_copy(src_h, src, n, i), src, sums) for i in range(NB)
               for n, (src_h, src, sums) in enumerate([(x_h, x, x_sums), (c_h, c, c_sums)])]
    for cp in [cp for _, cp, _, _ in rows_in] + first:
        cp.start()
    zero_ref[...] = jnp.zeros((8, 128), U32)
    for t in range(NT):
        ak[t, 0:PAD, :] = jnp.zeros((PAD, 128), U32)
    acc[...] = jnp.zeros(acc.shape, F32)
    for i, cp, src, sums in rows_in:
        cp.wait()
        mid = src.shape[1] // 2
        terms = _word_terms(_lhs_terms, LHS_PLAIN, *[
            src[_half(2 * i + u), cols] for u in range(2) for cols in (slice(0, mid), slice(mid, 2 * mid))])
        for k, n in enumerate(LHS_SUMS):
            sums[k, _half(i), :] = terms[n]
    for cp in first:
        cp.wait()
    shift = shift_v[...].astype(F32)
    for t in range(NT):
        shift32[t, 0:4, :] = shift[:, _tile(t)]
    ssmd32[...] = ssmd_v[...].astype(F32) * 0.5
    aq_copy.start()

    def iteration(j, carry):
        @pl.when(j > 0)
        def _():
            for cp in weight_copies(j):
                cp.wait()

            @pl.when((j & 1) == 0)
            def _():
                for cp in ssm_copies(j >> 1):
                    cp.wait()

        @pl.when(j + 1 < NP)
        def _():
            for cp in weight_copies(j + 1):
                cp.start()

            @pl.when((j & 1) == 1)
            def _():
                for cp in ssm_copies((j >> 1) + 1):
                    cp.start()

        head_pair(j)
        return carry

    jax.lax.fori_loop(0, NP, iteration, 0)

    aq_copy.wait()
    gate = gate_v[...].astype(F32)
    stores = []
    for i in range(NB):
        rows, words = slice(i * BQ, (i + 1) * BQ), slice(i * BQ // 2, (i + 1) * BQ // 2)
        q = [_bf(aq[words, _tile(t)]).astype(F32) for t in range(NT)]
        logit = q[0] * gate[0:1, :]
        for t in range(1, NT):
            logit = logit + q[t] * gate[t:t + 1, :]
        g = jax.nn.sigmoid(jnp.sum(logit, axis=1, keepdims=True))
        for t in range(NT):
            a = q[t] * _bf(y_buf[words, _tile(t)]).astype(F32)
            out_v[rows, _tile(t)] = (g * a + (1.0 - g) * acc[rows, _tile(t)]).astype(BF)
        stores.append(copy(out_v.at[pl.ds(i * BQ, BQ)], out_h.at[pl.ds(i * BQ, BQ)], sem_o.at[i]))
        stores[-1].start()
    for cp in stores:
        cp.wait()


@jax.jit
def pallas_gated_mix__ssm_conv_h3__compressed_kv_cla__prompt_kernel(
        A_q, A_k, A_v, A_shift_k, A_ssm_k, A_ssm_D, B_x, B_c_kv, B_w_q, B_w_uk, B_w_uv, B_w_o, gate_w):
    vmem, dma = pltpu.VMEM, pltpu.SemaphoreType.DMA
    scratch = [
        vmem((S // 2, D), U32), vmem((NT, PAD + S // 2, 128), U32), vmem((NT, S // 2, 128), U32),
        vmem((NT, HW, S), U32),
        vmem((S // 2, D), U32), vmem((S // 2, DC), U32),
        vmem((5, NB * HW, D // 2), U32), vmem((5, NB * HW, DC // 2), U32),
        vmem((2, D, HD), U32), vmem((2, DC, HD), U32), vmem((2, DC, HD), U32), vmem((2, HD, D), U32),
        vmem((S, 128), F32), vmem((S // 2, D), U32), vmem((S, D), F32), vmem((S, D), BF),
        vmem((4, D), BF), vmem((NT, 128), BF), vmem((NT, 128), BF), vmem((NT, 8, 128), F32), vmem((NT, 128), F32),
        vmem((2, 3, HF, C), U32), vmem((8, 128), U32),
        dma((3, NT)), dma((2, NB)), dma((2, 4)), dma((5,)), dma((NB,)),
    ]
    out = pl.pallas_call(
        _kernel,
        out_shape=jax.ShapeDtypeStruct((S, D), BF),
        in_specs=[pl.BlockSpec(memory_space=pl.ANY)] * 14,
        out_specs=pl.BlockSpec(memory_space=pl.ANY),
        scratch_shapes=scratch,
        compiler_params=pltpu.CompilerParams(vmem_limit_bytes=110 * 1024 * 1024, disable_bounds_checks=True),
    )(A_q.reshape(S, D), A_k.reshape(S, D), A_v.reshape(S, D), A_shift_k.T, A_ssm_k, A_ssm_D.reshape(NT, 128),
      B_x.reshape(S, D), B_c_kv.reshape(S, DC), B_w_q, B_w_uk, B_w_uv, B_w_o.reshape(NP, 2 * HD, D),
      gate_w.reshape(NT, 128), jnp.asarray(_DFT))
    return out.reshape(1, S, D)
```

```python
import functools

import numpy as np
import jax
import jax.numpy as jnp
import jax.experimental.pallas as pl
import jax.experimental.pallas.tpu as pltpu

S, D, H, HD, DC = 2048, 1024, 32, 128, 512
NT, NTC = D // 128, DC // 128
NP = H // 2
BQ = 256
NB = S // BQ
HW = 64
C = 128
NC = S // C
HF = C // 2
MB = 4
PAD = 8

FWD_AT = 1
FWD_SPAN = 3
MAC_END = 9
INV_AT = 11
PACED_FROM = 9
MAC_LAG = 24
KV_LAG = 14
EXP_LAG = 11
ORDER = [6, 0, 3, 4, 2, 1, 5]

LOG2E = 1.4426950408889634
QSCALE = (HD ** -0.5) * LOG2E
MASKED = -1e9 * LOG2E
BF, F32, U32 = jnp.bfloat16, jnp.float32, jnp.uint32


def _dft_words():
    t_nat = np.arange(C, dtype=np.float64)
    t_par = np.concatenate([t_nat[0::2], t_nat[1::2]])
    mats = []
    for h in range(2):
        f = 2.0 * np.arange(h * HF, (h + 1) * HF, dtype=np.float64) + 0.5
        row = []
        for t in (t_nat, t_par):
            ang = 2.0 * np.pi * np.outer(f, t) / (2 * C)
            row.append(np.concatenate([np.cos(ang), -np.sin(ang)], axis=0))
        ang = 2.0 * np.pi * np.outer(t_par + C, f) / (2 * C)
        row.append(np.concatenate([np.cos(ang), -np.sin(ang)], axis=1) / C)
        mats.append(np.stack(row))
    bits = np.stack(mats).astype(np.float32).view(np.uint32)
    bits = (bits + np.uint32(0x7FFF) + ((bits >> np.uint32(16)) & np.uint32(1))) >> np.uint32(16)
    return (bits[:, :, 0::2, :] | (bits[:, :, 1::2, :] << np.uint32(16))).astype(np.uint32)


_DFT = _dft_words()


def _mm(a, b):
    return jnp.dot(a, b, preferred_element_type=F32)


def _mm_nt(a, b):
    return jax.lax.dot_general(a, b, (((1,), (1,)), ((), ())), preferred_element_type=F32)


def _bf(words):
    return pltpu.bitcast(words, BF)


def _lo(words):
    return pltpu.bitcast(words << 16, F32)


def _hi(words):
    return pltpu.bitcast(words & jnp.uint32(0xFFFF0000), F32)


def _pack(even_rows, odd_rows):
    return pltpu.pack_elementwise([even_rows, odd_rows], packed_dtype=BF)


def _lhs_terms(a11, a12, a21, a22):
    return [a11 + a22, a21 + a22, a11, a22, a11 + a12, a21 - a11, a12 - a22]


def _rhs_terms(b11, b12, b21, b22):
    return [b11 + b22, b11, b12 - b22, b21 - b11, b22, b11 + b12, b21 + b22]


def _combine(m):
    return m[0] + m[3] - m[4] + m[6], m[2] + m[4], m[1] + m[3], m[0] - m[1] + m[2] + m[5]


LHS_PLAIN = {2: 0, 3: 3}
RHS_PLAIN = {1: 0, 4: 3}
LHS_SUMS = [n for n in range(7) if n not in LHS_PLAIN]


def _word_terms(terms, plain, *words):
    lo, hi = terms(*[_lo(w) for w in words]), terms(*[_hi(w) for w in words])
    return [words[plain[n]] if n in plain else _pack(lo[n], hi[n]) for n in range(7)]


def _merge(a, b):
    out, i, k = [], 0, 0
    while i < len(a) or k < len(b):
        if k >= len(b) or (i < len(a) and (i + 1) * len(b) <= (k + 1) * len(a)):
            out.append(a[i])
            i += 1
        else:
            out.append(b[k])
            k += 1
    return out


def _tile(n):
    return slice(n * 128, (n + 1) * 128)


def _half(n):
    return slice(n * HW, (n + 1) * HW)


def _kernel(aq_h, ak_h, av_h, shift_h, sk_h, ssmd_h, x_h, c_h, wq_h, wuk_h, wuv_h, wo_h, gate_h, dft_h, out_h,
            aq, ak, av, sk, x, c, x_sums, c_sums, wq, wk, wv, wo, y_half, y_buf, acc, out_v,
            shift_v, ssmd_v, gate_v, shift32, ssmd32, dft, zero_ref,
            sem_a, sem_x, sem_w, sem_s, sem_o):
    P = functools.partial
    copy = pltpu.make_async_copy

    def ssm_copies(i):
        cols = pl.ds(i * 128, 128)
        return [copy(ak_h.bitcast(U32).at[:, cols], ak.at[i, pl.ds(PAD, S // 2)], sem_a.at[0, i]),
                copy(av_h.bitcast(U32).at[:, cols], av.at[i], sem_a.at[1, i]),
                copy(sk_h.bitcast(U32).at[pl.ds(i * HW, HW), :], sk.at[i], sem_a.at[2, i])]

    def row_copy(src, dst, n, i):
        rows = pl.ds(i * BQ // 2, BQ // 2)
        return copy(src.bitcast(U32).at[rows], dst.at[rows], sem_x.at[n, i])

    def weight_copies(j):
        slot = j & 1
        cps = [copy(src.bitcast(U32).at[:, j, :], dst.at[slot], sem_w.at[slot, n])
               for n, (src, dst) in enumerate([(wq_h, wq), (wuk_h, wk), (wuv_h, wv)])]
        return cps + [copy(wo_h.bitcast(U32).at[j], wo.at[slot], sem_w.at[slot, 3])]

    aq_copy = copy(aq_h.bitcast(U32), aq, sem_s.at[4])

    def head_pair(j):
        slot = j & 1
        ti = j >> 1
        zero = zero_ref[...]
        causal = (jax.lax.broadcasted_iota(jnp.int32, (128, 128), 1) <=
                  jax.lax.broadcasted_iota(jnp.int32, (128, 128), 0))
        issued = []

        def token(lag):
            return zero & pltpu.bitcast(issued[max(len(issued) - lag, 0)][0:8, :], U32)

        def after(v, tok):
            return pltpu.bitcast(pltpu.bitcast(v, U32) | tok, F32)

        k_spec, x_spec, kv, y_spec = {}, {}, {}, {}

        def transform_filter(m):
            k_spec[m] = _mm_nt(_bf(dft[slot, 0]), _bf(sk[ti, :, _tile(m)]))
            return k_spec[m]

        def transform_input(n):
            r0 = PAD + n * HW
            w0, w1, w2 = (ak[ti, r0 - d:r0 - d + HW, :] for d in range(3))
            tok = token(KV_LAG)
            s0, s1, s2, s3 = (
                jnp.concatenate([after(jnp.broadcast_to(shift32[ti, d:d + 1, :], (8, 128)), tok)] * (HW // 8), axis=0)
                for d in range(4))
            e0, o0, e1, o1, o2 = _lo(w0), _hi(w0), _lo(w1), _hi(w1), _hi(w2)
            v = av[ti, _half(n), :]
            kv[n] = jnp.concatenate([(e0 * s0 + o1 * s1 + e1 * s2 + o2 * s3) * _lo(v),
                                     (o0 * s0 + e0 * s1 + o1 * s2 + e1 * s3) * _hi(v)], axis=0)
            x_spec[n] = _mm(_bf(dft[slot, 1]), kv[n].astype(BF))
            return x_spec[n]

        def spectral_product():
            for r in range(HF // 8):
                re, im = slice(r * 8, r * 8 + 8), slice(HF + r * 8, HF + r * 8 + 8)
                for b in range(NC // MB):
                    acc_re, acc_im = [None] * MB, [None] * MB
                    for n in range((b + 1) * MB):
                        tok = yield
                        xr, xi = after(x_spec[n][re, :], tok), after(x_spec[n][im, :], tok)
                        for u in range(MB):
                            m = b * MB + u - n
                            if m >= 0:
                                kr, ki = k_spec[m][re, :], k_spec[m][im, :]
                                pr, pi = xr * kr - xi * ki, xr * ki + xi * kr
                                acc_re[u] = pr if n == 0 else acc_re[u] + pr
                                acc_im[u] = pi if n == 0 else acc_im[u] + pi
                                y_spec[(b * MB + u, r)] = (acc_re[u], acc_im[u])
                        yield acc_im[MB - 1]

        def transform_back(n):
            cur = [y_spec[(n, r)] for r in range(HF // 8)]
            if n == 0:
                parts = [im for _, im in cur] + [-re for re, _ in cur]
            else:
                old = [y_spec[(n - 1, r)] for r in range(HF // 8)]
                parts = [o[0] + v[1] for o, v in zip(old, cur)] + [o[1] - v[0] for o, v in zip(old, cur)]
            conv = _mm(_bf(dft[slot, 2]), jnp.concatenate(parts, axis=0).astype(BF))
            y = conv + kv[n] * ssmd32[pl.ds(ti, 1), :] + jnp.where(slot == 1, y_half[_tile(n), :], 0.0)
            y_half[_tile(n), :] = y
            y_buf[_half(n), pl.ds(pl.multiple_of(ti * 128, 128), 128)] = _pack(y[0:HW, :], y[HW:, :])
            return conv

        qs, ks, vs, ctx, rhs = {}, {}, {}, {}, {}

        def project(i, name):
            src, sums, nt, w = {"q": (x, x_sums, NT // 2, wq), "k": (c, c_sums, NTC // 2, wk),
                                "v": (c, c_sums, NTC // 2, wv)}[name]
            m = [None] * 7

            def step(n, t):
                if (name, t) not in rhs:
                    top, bot = w[slot, _tile(t), :], w[slot, _tile(t + nt), :]
                    rhs[(name, t)] = [v.astype(BF) for v in _rhs_terms(_lo(top), _hi(top), _lo(bot), _hi(bot))]
                if n in LHS_PLAIN:
                    h = LHS_PLAIN[n] // 3
                    lhs = src[_half(2 * i + h), _tile(t + h * nt)]
                else:
                    lhs = sums[LHS_SUMS.index(n), _half(i), _tile(t)]
                d = _mm(_bf(lhs), rhs[(name, t)][n])
                m[n] = d if t == 0 else m[n] + d
                if n == ORDER[-1] and t == nt - 1:
                    c11, c12, c21, c22 = _combine(m)
                    for e, (top, bot) in enumerate([(c11, c21), (c12, c22)]):
                        if name == "q":
                            top, bot = (top * QSCALE).astype(BF), (bot * QSCALE).astype(BF)
                            qs[(e, i, 0)] = jnp.concatenate([top, bot], axis=0)
                            qs[(e, i, 1)] = bot
                        else:
                            dst = ks if name == "k" else vs
                            dst[(e, 2 * i)], dst[(e, 2 * i + 1)] = top.astype(BF), bot.astype(BF)
                return d
            return [P(step, n, t) for n in ORDER for t in range(nt)]

        def key_tiles(i):
            return [(0, t) for t in range(2 * i + 1)] + [(1, 2 * i + 1)]

        def scores(i, e, st):
            def step(u0, t):
                s = _mm_nt(qs[(e, i, u0)], ks[(e, t)])
                for u in range(u0, 2):
                    part = s[_tile(u - u0), :]
                    if t == 2 * i + u:
                        part = jnp.where(causal, part, MASKED)
                    st["s"][(u, t)] = part
                    st["max"][u] = part if t == 0 else jnp.maximum(st["max"][u], part)
                    if t == 2 * i + u:
                        st["max"][u] = jnp.max(st["max"][u], axis=1, keepdims=True)
                return s
            return [P(step, u0, t) for u0, t in key_tiles(i)]

        def attend(i, e, st):
            def step(u0, t):
                tok = token(EXP_LAG) if 2 * i + e >= PACED_FROM else None
                probs = []
                for u in range(u0, 2):
                    m = st["max"][u]
                    if tok is not None:
                        m = jnp.broadcast_to(m, (128, 128))
                        m = jnp.concatenate([after(m[8 * n:8 * n + 8, :], tok) for n in range(16)], axis=0)
                    p = jnp.exp2(st["s"].pop((u, t)) - m)
                    st["sum"][u] = p if t == 0 else st["sum"][u] + p
                    probs.append(p.astype(BF))
                d = _mm(jnp.concatenate(probs, axis=0), vs[(e, t)])
                for u in range(u0, 2):
                    part = d[_tile(u - u0), :]
                    st["out"][u] = part if t == 0 else st["out"][u] + part
                if u0 == 1:
                    for u in range(2):
                        total = jnp.sum(st["sum"][u], axis=1, keepdims=True)
                        r = pl.reciprocal(total, approx=True)
                        ctx[(e, i, u)] = st["out"][u] * (r * (2.0 - total * r))
                return d
            return [P(step, u0, t) for u0, t in key_tiles(i)]

        def project_out(i):
            lhs, m = [], [None] * 7

            def step(t, n):
                left, right = _tile(t), _tile(t + NT // 2)
                if ("o", t) not in rhs:
                    rhs[("o", t)] = _word_terms(_rhs_terms, RHS_PLAIN, *[
                        wo[slot, _half(e), cols] for e in range(2) for cols in (left, right)])
                if not lhs:
                    lhs.extend(v.astype(BF) for v in _lhs_terms(
                        ctx[(0, i, 0)], ctx[(1, i, 0)], ctx[(0, i, 1)], ctx[(1, i, 1)]))
                m[n] = _mm(lhs[n], _bf(rhs[("o", t)][n]))
                if n == ORDER[-1]:
                    blocks = [(_tile(2 * i + u), cols) for u in range(2) for cols in (left, right)]
                    for block, v in zip(blocks, _combine(m)):
                        acc[block] += v
                return m[n]
            return [P(step, t, n) for t in range(NT // 2) for n in ORDER]

        units = [(i, e) for i in range(NB) for e in range(2)]
        states = [dict(s={}, max=[None] * 2, sum=[None] * 2, out=[None] * 2) for _ in units]
        extra = {FWD_AT + n: [P(transform_input, k) for k in range(n * NC // FWD_SPAN, (n + 1) * NC // FWD_SPAN)]
                 for n in range(FWD_SPAN)}
        extra[INV_AT] = [P(transform_back, n) for n in range(NC)]
        seq = [P(transform_filter, m) for m in range(NC)]
        seq += project(0, "k") + project(0, "q") + project(0, "v") + scores(*units[0], states[0])
        ends = []
        for n, (i, e) in enumerate(units):
            if n + 1 < len(units):
                seq += scores(*units[n + 1], states[n + 1])
            if i + 1 == NB:
                fill = project_out(i - 2 + e)
            elif e == 0:
                fill = project(i + 1, "q") + project(i + 1, "k")
            else:
                fill = (project_out(i - 2) if i >= 2 else []) + project(i + 1, "v")
            seq += _merge(_merge(fill, extra.get(n, [])), attend(i, e, states[n]))
            ends.append(len(seq))
        seq += project_out(NB - 1)

        product = spectral_product()
        steps = (HF // 8) * sum((b + 1) * MB for b in range(NC // MB))
        lo, hi = ends[FWD_AT + FWD_SPAN - 1], ends[MAC_END]
        done, last = 0, None
        for k, item in enumerate(seq):
            while k >= lo and done < steps and done * (hi - lo) < (k - lo + 1) * steps:
                next(product)
                tok = token(MAC_LAG)
                last = product.send(tok if last is None else tok & pltpu.bitcast(last, U32))
                done += 1
            issued.append(item())

    first = weight_copies(0) + ssm_copies(0) + [
        copy(src, dst, sem_s.at[n]) for n, (src, dst) in enumerate(
            [(shift_h, shift_v), (ssmd_h, ssmd_v), (gate_h, gate_v), (dft_h, dft)])]
    rows_in = [(i, row_copy(src_h, src, n, i), src, sums) for i in range(NB)
               for n, (src_h, src, sums) in enumerate([(x_h, x, x_sums), (c_h, c, c_sums)])]
    for cp in [cp for _, cp, _, _ in rows_in] + first:
        cp.start()
    zero_ref[...] = jnp.zeros((8, 128), U32)
    for t in range(NT):
        ak[t, 0:PAD, :] = jnp.zeros((PAD, 128), U32)
    acc[...] = jnp.zeros(acc.shape, F32)
    y_half[...] = jnp.zeros(y_half.shape, F32)
    for i, cp, src, sums in rows_in:
        cp.wait()
        mid = src.shape[1] // 2
        terms = _word_terms(_lhs_terms, LHS_PLAIN, *[
            src[_half(2 * i + u), cols] for u in range(2) for cols in (slice(0, mid), slice(mid, 2 * mid))])
        for k, n in enumerate(LHS_SUMS):
            sums[k, _half(i), :] = terms[n]
    for cp in first:
        cp.wait()
    shift = shift_v[...].astype(F32)
    for t in range(NT):
        shift32[t, 0:4, :] = shift[:, _tile(t)]
    ssmd32[...] = ssmd_v[...].astype(F32) * 0.5
    aq_copy.start()

    def iteration(j, carry):
        @pl.when(j > 0)
        def _():
            for cp in weight_copies(j):
                cp.wait()

            @pl.when((j & 1) == 0)
            def _():
                for cp in ssm_copies(j >> 1):
                    cp.wait()

        @pl.when(j + 1 < NP)
        def _():
            for cp in weight_copies(j + 1):
                cp.start()

            @pl.when((j & 1) == 1)
            def _():
                for cp in ssm_copies((j >> 1) + 1):
                    cp.start()

        head_pair(j)
        return carry

    jax.lax.fori_loop(0, NP, iteration, 0)

    aq_copy.wait()
    gate = gate_v[...].astype(F32)
    stores = []
    for i in range(NB):
        rows, words = slice(i * BQ, (i + 1) * BQ), slice(i * BQ // 2, (i + 1) * BQ // 2)
        q = [_bf(aq[words, _tile(t)]).astype(F32) for t in range(NT)]
        logit = q[0] * gate[0:1, :]
        for t in range(1, NT):
            logit = logit + q[t] * gate[t:t + 1, :]
        g = jax.nn.sigmoid(jnp.sum(logit, axis=1, keepdims=True))
        for t in range(NT):
            a = q[t] * _bf(y_buf[words, _tile(t)]).astype(F32)
            out_v[rows, _tile(t)] = (g * a + (1.0 - g) * acc[rows, _tile(t)]).astype(BF)
        stores.append(copy(out_v.at[pl.ds(i * BQ, BQ)], out_h.at[pl.ds(i * BQ, BQ)], sem_o.at[i]))
        stores[-1].start()
    for cp in stores:
        cp.wait()


@jax.jit
def pallas_gated_mix__ssm_conv_h3__compressed_kv_cla__prompt_kernel(
        A_q, A_k, A_v, A_shift_k, A_ssm_k, A_ssm_D, B_x, B_c_kv, B_w_q, B_w_uk, B_w_uv, B_w_o, gate_w):
    vmem, dma = pltpu.VMEM, pltpu.SemaphoreType.DMA
    scratch = [
        vmem((S // 2, D), U32), vmem((NT, PAD + S // 2, 128), U32), vmem((NT, S // 2, 128), U32),
        vmem((NT, HW, S), U32),
        vmem((S // 2, D), U32), vmem((S // 2, DC), U32),
        vmem((5, NB * HW, D // 2), U32), vmem((5, NB * HW, DC // 2), U32),
        vmem((2, D, HD), U32), vmem((2, DC, HD), U32), vmem((2, DC, HD), U32), vmem((2, HD, D), U32),
        vmem((S, 128), F32), vmem((S // 2, D), U32), vmem((S, D), F32), vmem((S, D), BF),
        vmem((4, D), BF), vmem((NT, 128), BF), vmem((NT, 128), BF), vmem((NT, 8, 128), F32), vmem((NT, 128), F32),
        vmem((2, 3, HF, C), U32), vmem((8, 128), U32),
        dma((3, NT)), dma((2, NB)), dma((2, 4)), dma((5,)), dma((NB,)),
    ]
    out = pl.pallas_call(
        _kernel,
        out_shape=jax.ShapeDtypeStruct((S, D), BF),
        in_specs=[pl.BlockSpec(memory_space=pl.ANY)] * 14,
        out_specs=pl.BlockSpec(memory_space=pl.ANY),
        scratch_shapes=scratch,
        compiler_params=pltpu.CompilerParams(vmem_limit_bytes=110 * 1024 * 1024, disable_bounds_checks=True),
    )(A_q.reshape(S, D), A_k.reshape(S, D), A_v.reshape(S, D), A_shift_k.T, A_ssm_k, A_ssm_D.reshape(NT, 128),
      B_x.reshape(S, D), B_c_kv.reshape(S, DC), B_w_q, B_w_uk, B_w_uv, B_w_o.reshape(NP, 2 * HD, D),
      gate_w.reshape(NT, 128), jnp.asarray(_DFT))
    return out.reshape(1, S, D)
```

```python
import functools

import numpy as np
import jax
import jax.numpy as jnp
import jax.experimental.pallas as pl
import jax.experimental.pallas.tpu as pltpu

S, D, H, HD, DC = 2048, 1024, 32, 128, 512
NT, NTC = D // 128, DC // 128
NP = H // 2
BQ = 256
NB = S // BQ
HW = 64
C = 128
NC = S // C
HF = C // 2
MB = 4
PAD = 8

FWD_AT = 1
FWD_SPAN = 3
MAC_END = 9
INV_AT = 11
PACED_FROM = 9
MAC_LAG = 24
KV_LAG = 14
EXP_LAG = 11
ORDER = [6, 0, 3, 4, 2, 1, 5]

LOG2E = 1.4426950408889634
QSCALE = (HD ** -0.5) * LOG2E
MASKED = -1e9 * LOG2E
BF, F32, U32 = jnp.bfloat16, jnp.float32, jnp.uint32


def _dft_words():
    t_nat = np.arange(C, dtype=np.float64)
    t_par = np.concatenate([t_nat[0::2], t_nat[1::2]])
    mats = []
    for h in range(2):
        f = 2.0 * np.arange(h * HF, (h + 1) * HF, dtype=np.float64) + 0.5
        row = []
        for t in (t_nat, t_par):
            ang = 2.0 * np.pi * np.outer(f, t) / (2 * C)
            row.append(np.concatenate([np.cos(ang), -np.sin(ang)], axis=0))
        ang = 2.0 * np.pi * np.outer(t_par + C, f) / (2 * C)
        row.append(np.concatenate([np.cos(ang), -np.sin(ang)], axis=1) / C)
        mats.append(np.stack(row))
    bits = np.stack(mats).astype(np.float32).view(np.uint32)
    bits = (bits + np.uint32(0x7FFF) + ((bits >> np.uint32(16)) & np.uint32(1))) >> np.uint32(16)
    return (bits[:, :, 0::2, :] | (bits[:, :, 1::2, :] << np.uint32(16))).astype(np.uint32)


_DFT = _dft_words()


def _mm(a, b):
    return jnp.dot(a, b, preferred_element_type=F32)


def _mm_nt(a, b):
    return jax.lax.dot_general(a, b, (((1,), (1,)), ((), ())), preferred_element_type=F32)


def _bf(words):
    return pltpu.bitcast(words, BF)


def _lo(words):
    return pltpu.bitcast(words << 16, F32)


def _hi(words):
    return pltpu.bitcast(words & jnp.uint32(0xFFFF0000), F32)


def _pack(even_rows, odd_rows):
    return pltpu.pack_elementwise([even_rows, odd_rows], packed_dtype=BF)


def _lhs_terms(a11, a12, a21, a22):
    return [a11 + a22, a21 + a22, a11, a22, a11 + a12, a21 - a11, a12 - a22]


def _rhs_terms(b11, b12, b21, b22):
    return [b11 + b22, b11, b12 - b22, b21 - b11, b22, b11 + b12, b21 + b22]


def _combine(m):
    return m[0] + m[3] - m[4] + m[6], m[2] + m[4], m[1] + m[3], m[0] - m[1] + m[2] + m[5]


LHS_PLAIN = {2: 0, 3: 3}
RHS_PLAIN = {1: 0, 4: 3}
LHS_SUMS = [n for n in range(7) if n not in LHS_PLAIN]


def _word_terms(terms, plain, *words):
    lo, hi = terms(*[_lo(w) for w in words]), terms(*[_hi(w) for w in words])
    return [words[plain[n]] if n in plain else _pack(lo[n], hi[n]) for n in range(7)]


def _merge(a, b):
    out, i, k = [], 0, 0
    while i < len(a) or k < len(b):
        if k >= len(b) or (i < len(a) and (i + 1) * len(b) <= (k + 1) * len(a)):
            out.append(a[i])
            i += 1
        else:
            out.append(b[k])
            k += 1
    return out


def _tile(n):
    return slice(n * 128, (n + 1) * 128)


def _half(n):
    return slice(n * HW, (n + 1) * HW)


def _kernel(x_h, ak_h, av_h, shift_h, sk_h, ssmd_h, c_h, wq_h, wuk_h, wuv_h, wo_h, gate_h, dft_h, out_h,
            ak, av, sk, x, c, x_sums, c_sums, wq, wk, wv, wo, y_half, y_buf, acc, out_v,
            shift_v, ssmd_v, gate_v, shift32, ssmd32, dft, zero_ref,
            sem_a, sem_x, sem_w, sem_s, sem_o):
    P = functools.partial
    copy = pltpu.make_async_copy

    def ssm_copies(i):
        cols = pl.ds(i * 128, 128)
        return [copy(ak_h.bitcast(U32).at[:, cols], ak.at[i, pl.ds(PAD, S // 2)], sem_a.at[0, i]),
                copy(av_h.bitcast(U32).at[:, cols], av.at[i], sem_a.at[1, i]),
                copy(sk_h.bitcast(U32).at[pl.ds(i * HW, HW), :], sk.at[i], sem_a.at[2, i])]

    def row_copy(src, dst, n, i):
        rows = pl.ds(i * BQ // 2, BQ // 2)
        return copy(src.bitcast(U32).at[rows], dst.at[rows], sem_x.at[n, i])

    def weight_copies(j):
        slot = j & 1
        cps = [copy(src.bitcast(U32).at[:, j, :], dst.at[slot], sem_w.at[slot, n])
               for n, (src, dst) in enumerate([(wq_h, wq), (wuk_h, wk), (wuv_h, wv)])]
        return cps + [copy(wo_h.bitcast(U32).at[j], wo.at[slot], sem_w.at[slot, 3])]

    def head_pair(j):
        slot = j & 1
        ti = j >> 1
        zero = zero_ref[...]
        causal = (jax.lax.broadcasted_iota(jnp.int32, (128, 128), 1) <=
                  jax.lax.broadcasted_iota(jnp.int32, (128, 128), 0))
        issued = []

        def token(lag):
            return zero & pltpu.bitcast(issued[max(len(issued) - lag, 0)][0:8, :], U32)

        def after(v, tok):
            return pltpu.bitcast(pltpu.bitcast(v, U32) | tok, F32)

        k_spec, x_spec, kv, y_spec = {}, {}, {}, {}

        def transform_filter(m):
            k_spec[m] = _mm_nt(_bf(dft[slot, 0]), _bf(sk[ti, :, _tile(m)]))
            return k_spec[m]

        def transform_input(n):
            r0 = PAD + n * HW
            w0, w1, w2 = (ak[ti, r0 - d:r0 - d + HW, :] for d in range(3))
            tok = token(KV_LAG)
            s0, s1, s2, s3 = (
                jnp.concatenate([after(jnp.broadcast_to(shift32[ti, d:d + 1, :], (8, 128)), tok)] * (HW // 8), axis=0)
                for d in range(4))
            e0, o0, e1, o1, o2 = _lo(w0), _hi(w0), _lo(w1), _hi(w1), _hi(w2)
            v = av[ti, _half(n), :]
            kv[n] = jnp.concatenate([(e0 * s0 + o1 * s1 + e1 * s2 + o2 * s3) * _lo(v),
                                     (o0 * s0 + e0 * s1 + o1 * s2 + e1 * s3) * _hi(v)], axis=0)
            x_spec[n] = _mm(_bf(dft[slot, 1]), kv[n].astype(BF))
            return x_spec[n]

        def spectral_product():
            for r in range(HF // 8):
                re, im = slice(r * 8, r * 8 + 8), slice(HF + r * 8, HF + r * 8 + 8)
                for b in range(NC // MB):
                    acc_re, acc_im = [None] * MB, [None] * MB
                    for n in range((b + 1) * MB):
                        tok = yield
                        xr, xi = after(x_spec[n][re, :], tok), after(x_spec[n][im, :], tok)
                        for u in range(MB):
                            m = b * MB + u - n
                            if m >= 0:
                                kr, ki = k_spec[m][re, :], k_spec[m][im, :]
                                pr, pi = xr * kr - xi * ki, xr * ki + xi * kr
                                acc_re[u] = pr if n == 0 else acc_re[u] + pr
                                acc_im[u] = pi if n == 0 else acc_im[u] + pi
                                y_spec[(b * MB + u, r)] = (acc_re[u], acc_im[u])
                        yield acc_im[MB - 1]

        def transform_back(n):
            cur = [y_spec[(n, r)] for r in range(HF // 8)]
            if n == 0:
                parts = [im for _, im in cur] + [-re for re, _ in cur]
            else:
                old = [y_spec[(n - 1, r)] for r in range(HF // 8)]
                parts = [o[0] + v[1] for o, v in zip(old, cur)] + [o[1] - v[0] for o, v in zip(old, cur)]
            conv = _mm(_bf(dft[slot, 2]), jnp.concatenate(parts, axis=0).astype(BF))
            y = conv + kv[n] * ssmd32[pl.ds(ti, 1), :] + jnp.where(slot == 1, y_half[_tile(n), :], 0.0)
            y_half[_tile(n), :] = y
            y_buf[_half(n), pl.ds(pl.multiple_of(ti * 128, 128), 128)] = _pack(y[0:HW, :], y[HW:, :])
            return conv

        qs, ks, vs, ctx, rhs = {}, {}, {}, {}, {}

        def project(i, name):
            src, sums, nt, w = {"q": (x, x_sums, NT // 2, wq), "k": (c, c_sums, NTC // 2, wk),
                                "v": (c, c_sums, NTC // 2, wv)}[name]
            m = [None] * 7

            def step(n, t):
                if (name, t) not in rhs:
                    top, bot = w[slot, _tile(t), :], w[slot, _tile(t + nt), :]
                    rhs[(name, t)] = [v.astype(BF) for v in _rhs_terms(_lo(top), _hi(top), _lo(bot), _hi(bot))]
                if n in LHS_PLAIN:
                    h = LHS_PLAIN[n] // 3
                    lhs = src[_half(2 * i + h), _tile(t + h * nt)]
                else:
                    lhs = sums[LHS_SUMS.index(n), _half(i), _tile(t)]
                d = _mm(_bf(lhs), rhs[(name, t)][n])
                m[n] = d if t == 0 else m[n] + d
                if n == ORDER[-1] and t == nt - 1:
                    c11, c12, c21, c22 = _combine(m)
                    for e, (top, bot) in enumerate([(c11, c21), (c12, c22)]):
                        if name == "q":
                            top, bot = (top * QSCALE).astype(BF), (bot * QSCALE).astype(BF)
                            qs[(e, i, 0)] = jnp.concatenate([top, bot], axis=0)
                            qs[(e, i, 1)] = bot
                        else:
                            dst = ks if name == "k" else vs
                            dst[(e, 2 * i)], dst[(e, 2 * i + 1)] = top.astype(BF), bot.astype(BF)
                return d
            return [P(step, n, t) for n in ORDER for t in range(nt)]

        def key_tiles(i):
            return [(0, t) for t in range(2 * i + 1)] + [(1, 2 * i + 1)]

        def scores(i, e, st):
            def step(u0, t):
                s = _mm_nt(qs[(e, i, u0)], ks[(e, t)])
                for u in range(u0, 2):
                    part = s[_tile(u - u0), :]
                    if t == 2 * i + u:
                        part = jnp.where(causal, part, MASKED)
                    st["s"][(u, t)] = part
                    st["max"][u] = part if t == 0 else jnp.maximum(st["max"][u], part)
                    if t == 2 * i + u:
                        st["max"][u] = jnp.max(st["max"][u], axis=1, keepdims=True)
                return s
            return [P(step, u0, t) for u0, t in key_tiles(i)]

        def attend(i, e, st):
            def step(u0, t):
                tok = token(EXP_LAG) if 2 * i + e >= PACED_FROM else None
                probs = []
                for u in range(u0, 2):
                    m = st["max"][u]
                    if tok is not None:
                        m = jnp.broadcast_to(m, (128, 128))
                        m = jnp.concatenate([after(m[8 * n:8 * n + 8, :], tok) for n in range(16)], axis=0)
                    p = jnp.exp2(st["s"].pop((u, t)) - m)
                    st["sum"][u] = p if t == 0 else st["sum"][u] + p
                    probs.append(p.astype(BF))
                d = _mm(jnp.concatenate(probs, axis=0), vs[(e, t)])
                for u in range(u0, 2):
                    part = d[_tile(u - u0), :]
                    st["out"][u] = part if t == 0 else st["out"][u] + part
                if u0 == 1:
                    for u in range(2):
                        total = jnp.sum(st["sum"][u], axis=1, keepdims=True)
                        r = pl.reciprocal(total, approx=True)
                        ctx[(e, i, u)] = st["out"][u] * (r * (2.0 - total * r))
                return d
            return [P(step, u0, t) for u0, t in key_tiles(i)]

        def project_out(i):
            lhs, m = [], [None] * 7

            def step(t, n):
                left, right = _tile(t), _tile(t + NT // 2)
                if ("o", t) not in rhs:
                    rhs[("o", t)] = _word_terms(_rhs_terms, RHS_PLAIN, *[
                        wo[slot, _half(e), cols] for e in range(2) for cols in (left, right)])
                if not lhs:
                    lhs.extend(v.astype(BF) for v in _lhs_terms(
                        ctx[(0, i, 0)], ctx[(1, i, 0)], ctx[(0, i, 1)], ctx[(1, i, 1)]))
                m[n] = _mm(lhs[n], _bf(rhs[("o", t)][n]))
                if n == ORDER[-1]:
                    blocks = [(_tile(2 * i + u), cols) for u in range(2) for cols in (left, right)]
                    for block, v in zip(blocks, _combine(m)):
                        acc[block] += v
                return m[n]
            return [P(step, t, n) for t in range(NT // 2) for n in ORDER]

        units = [(i, e) for i in range(NB) for e in range(2)]
        states = [dict(s={}, max=[None] * 2, sum=[None] * 2, out=[None] * 2) for _ in units]
        extra = {FWD_AT + n: [P(transform_input, k) for k in range(n * NC // FWD_SPAN, (n + 1) * NC // FWD_SPAN)]
                 for n in range(FWD_SPAN)}
        extra[INV_AT] = [P(transform_back, n) for n in range(NC)]
        seq = [P(transform_filter, m) for m in range(NC)]
        seq += project(0, "k") + project(0, "q") + project(0, "v") + scores(*units[0], states[0])
        ends = []
        for n, (i, e) in enumerate(units):
            if n + 1 < len(units):
                seq += scores(*units[n + 1], states[n + 1])
            if i + 1 == NB:
                fill = project_out(i - 2 + e)
            elif e == 0:
                fill = project(i + 1, "q") + project(i + 1, "k")
            else:
                fill = (project_out(i - 2) if i >= 2 else []) + project(i + 1, "v")
            seq += _merge(_merge(fill, extra.get(n, [])), attend(i, e, states[n]))
            ends.append(len(seq))
        seq += project_out(NB - 1)

        product = spectral_product()
        steps = (HF // 8) * sum((b + 1) * MB for b in range(NC // MB))
        lo, hi = ends[FWD_AT + FWD_SPAN - 1], ends[MAC_END]
        done, last = 0, None
        for k, item in enumerate(seq):
            while k >= lo and done < steps and done * (hi - lo) < (k - lo + 1) * steps:
                next(product)
                tok = token(MAC_LAG)
                last = product.send(tok if last is None else tok & pltpu.bitcast(last, U32))
                done += 1
            issued.append(item())

    first = weight_copies(0) + ssm_copies(0) + [
        copy(src, dst, sem_s.at[n]) for n, (src, dst) in enumerate(
            [(shift_h, shift_v), (ssmd_h, ssmd_v), (gate_h, gate_v), (dft_h, dft)])]
    rows_in = [(i, row_copy(src_h, src, n, i), src, sums) for i in range(NB)
               for n, (src_h, src, sums) in enumerate([(x_h, x, x_sums), (c_h, c, c_sums)])]
    for cp in [cp for _, cp, _, _ in rows_in] + first:
        cp.start()
    zero_ref[...] = jnp.zeros((8, 128), U32)
    for t in range(NT):
        ak[t, 0:PAD, :] = jnp.zeros((PAD, 128), U32)
    acc[...] = jnp.zeros(acc.shape, F32)
    y_half[...] = jnp.zeros(y_half.shape, F32)
    for i, cp, src, sums in rows_in:
        cp.wait()
        mid = src.shape[1] // 2
        terms = _word_terms(_lhs_terms, LHS_PLAIN, *[
            src[_half(2 * i + u), cols] for u in range(2) for cols in (slice(0, mid), slice(mid, 2 * mid))])
        for k, n in enumerate(LHS_SUMS):
            sums[k, _half(i), :] = terms[n]
    for cp in first:
        cp.wait()
    shift = shift_v[...].astype(F32)
    for t in range(NT):
        shift32[t, 0:4, :] = shift[:, _tile(t)]
    ssmd32[...] = ssmd_v[...].astype(F32) * 0.5

    def iteration(j, carry):
        @pl.when(j > 0)
        def _():
            for cp in weight_copies(j):
                cp.wait()

            @pl.when((j & 1) == 0)
            def _():
                for cp in ssm_copies(j >> 1):
                    cp.wait()

        @pl.when(j + 1 < NP)
        def _():
            for cp in weight_copies(j + 1):
                cp.start()

            @pl.when((j & 1) == 1)
            def _():
                for cp in ssm_copies((j >> 1) + 1):
                    cp.start()

        head_pair(j)
        return carry

    jax.lax.fori_loop(0, NP, iteration, 0)

    gate = gate_v[...].astype(F32)
    stores = []
    for i in range(NB):
        rows, words = slice(i * BQ, (i + 1) * BQ), slice(i * BQ // 2, (i + 1) * BQ // 2)
        q = [_bf(x[words, _tile(t)]).astype(F32) for t in range(NT)]
        logit = q[0] * gate[0:1, :]
        for t in range(1, NT):
            logit = logit + q[t] * gate[t:t + 1, :]
        g = jax.nn.sigmoid(jnp.sum(logit, axis=1, keepdims=True))
        for t in range(NT):
            a = q[t] * _bf(y_buf[words, _tile(t)]).astype(F32)
            out_v[rows, _tile(t)] = (g * a + (1.0 - g) * acc[rows, _tile(t)]).astype(BF)
        stores.append(copy(out_v.at[pl.ds(i * BQ, BQ)], out_h.at[pl.ds(i * BQ, BQ)], sem_o.at[i]))
        stores[-1].start()
    for cp in stores:
        cp.wait()


@jax.jit
def pallas_gated_mix__ssm_conv_h3__compressed_kv_cla__prompt_kernel(
        A_q, A_k, A_v, A_shift_k, A_ssm_k, A_ssm_D, B_x, B_c_kv, B_w_q, B_w_uk, B_w_uv, B_w_o, gate_w):
    del B_x
    vmem, dma = pltpu.VMEM, pltpu.SemaphoreType.DMA
    scratch = [
        vmem((NT, PAD + S // 2, 128), U32), vmem((NT, S // 2, 128), U32),
        vmem((NT, HW, S), U32),
        vmem((S // 2, D), U32), vmem((S // 2, DC), U32),
        vmem((5, NB * HW, D // 2), U32), vmem((5, NB * HW, DC // 2), U32),
        vmem((2, D, HD), U32), vmem((2, DC, HD), U32), vmem((2, DC, HD), U32), vmem((2, HD, D), U32),
        vmem((S, 128), F32), vmem((S // 2, D), U32), vmem((S, D), F32), vmem((S, D), BF),
        vmem((4, D), BF), vmem((NT, 128), BF), vmem((NT, 128), BF), vmem((NT, 8, 128), F32), vmem((NT, 128), F32),
        vmem((2, 3, HF, C), U32), vmem((8, 128), U32),
        dma((3, NT)), dma((2, NB)), dma((2, 4)), dma((4,)), dma((NB,)),
    ]
    out = pl.pallas_call(
        _kernel,
        out_shape=jax.ShapeDtypeStruct((S, D), BF),
        in_specs=[pl.BlockSpec(memory_space=pl.ANY)] * 13,
        out_specs=pl.BlockSpec(memory_space=pl.ANY),
        scratch_shapes=scratch,
        compiler_params=pltpu.CompilerParams(vmem_limit_bytes=110 * 1024 * 1024, disable_bounds_checks=True),
    )(A_q.reshape(S, D), A_k.reshape(S, D), A_v.reshape(S, D), A_shift_k.T, A_ssm_k, A_ssm_D.reshape(NT, 128),
      B_c_kv.reshape(S, DC), B_w_q, B_w_uk, B_w_uv, B_w_o.reshape(NP, 2 * HD, D),
      gate_w.reshape(NT, 128), jnp.asarray(_DFT))
    return out.reshape(1, S, D)
```

```python
import functools

import numpy as np
import jax
import jax.numpy as jnp
import jax.experimental.pallas as pl
import jax.experimental.pallas.tpu as pltpu

S, D, H, HD, DC = 2048, 1024, 32, 128, 512
NT, NTC = D // 128, DC // 128
NP = H // 2
BQ = 256
NB = S // BQ
HW = 64
C = 128
NC = S // C
HF = C // 2
MB = 4
PAD = 8

FWD_AT = 1
FWD_SPAN = 3
MAC_END = 9
INV_AT = 11
PACED_FROM = 9
MAC_LAG = 24
KV_LAG = 14
EXP_LAG = 11
ORDER = [6, 0, 3, 4, 2, 1, 5]

LOG2E = 1.4426950408889634
QSCALE = (HD ** -0.5) * LOG2E
MASKED = -1e9 * LOG2E
BF, F32, U32 = jnp.bfloat16, jnp.float32, jnp.uint32


def _dft_words():
    t_nat = np.arange(C, dtype=np.float64)
    t_par = np.concatenate([t_nat[0::2], t_nat[1::2]])
    mats = []
    for h in range(2):
        f = 2.0 * np.arange(h * HF, (h + 1) * HF, dtype=np.float64) + 0.5
        row = []
        for t in (t_nat, t_par):
            ang = 2.0 * np.pi * np.outer(f, t) / (2 * C)
            row.append(np.concatenate([np.cos(ang), -np.sin(ang)], axis=0))
        ang = 2.0 * np.pi * np.outer(t_par + C, f) / (2 * C)
        row.append(np.concatenate([np.cos(ang), -np.sin(ang)], axis=1) / C)
        mats.append(np.stack(row))
    bits = np.stack(mats).astype(np.float32).view(np.uint32)
    bits = (bits + np.uint32(0x7FFF) + ((bits >> np.uint32(16)) & np.uint32(1))) >> np.uint32(16)
    return (bits[:, :, 0::2, :] | (bits[:, :, 1::2, :] << np.uint32(16))).astype(np.uint32)


_DFT = _dft_words()


def _mm(a, b):
    return jnp.dot(a, b, preferred_element_type=F32)


def _mm_nt(a, b):
    return jax.lax.dot_general(a, b, (((1,), (1,)), ((), ())), preferred_element_type=F32)


def _bf(words):
    return pltpu.bitcast(words, BF)


def _lo(words):
    return pltpu.bitcast(words << 16, F32)


def _hi(words):
    return pltpu.bitcast(words & jnp.uint32(0xFFFF0000), F32)


def _pack(even_rows, odd_rows):
    return pltpu.pack_elementwise([even_rows, odd_rows], packed_dtype=BF)


def _lhs_terms(a11, a12, a21, a22):
    return [a11 + a22, a21 + a22, a11, a22, a11 + a12, a21 - a11, a12 - a22]


def _rhs_terms(b11, b12, b21, b22):
    return [b11 + b22, b11, b12 - b22, b21 - b11, b22, b11 + b12, b21 + b22]


def _combine(m):
    return m[0] + m[3] - m[4] + m[6], m[2] + m[4], m[1] + m[3], m[0] - m[1] + m[2] + m[5]


LHS_PLAIN = {2: 0, 3: 3}
RHS_PLAIN = {1: 0, 4: 3}
LHS_SUMS = [n for n in range(7) if n not in LHS_PLAIN]


def _word_terms(terms, plain, *words):
    lo, hi = terms(*[_lo(w) for w in words]), terms(*[_hi(w) for w in words])
    return [words[plain[n]] if n in plain else _pack(lo[n], hi[n]) for n in range(7)]


def _merge(a, b):
    out, i, k = [], 0, 0
    while i < len(a) or k < len(b):
        if k >= len(b) or (i < len(a) and (i + 1) * len(b) <= (k + 1) * len(a)):
            out.append(a[i])
            i += 1
        else:
            out.append(b[k])
            k += 1
    return out


def _tile(n):
    return slice(n * 128, (n + 1) * 128)


def _half(n):
    return slice(n * HW, (n + 1) * HW)


def _kernel(x_h, ak_h, av_h, shift_h, sk_h, ssmd_h, c_h, wq_h, wuk_h, wuv_h, wo_h, gate_h, dft_h, out_h,
            ak, av, sk, x, c, x_sums, c_sums, wq, wk, wv, wo, y_half, y_buf, acc, out_v, gates,
            shift_v, ssmd_v, gate_v, shift32, ssmd32, dft, zero_ref,
            sem_a, sem_x, sem_w, sem_s, sem_o):
    P = functools.partial
    copy = pltpu.make_async_copy

    def ssm_copies(i):
        cols = pl.ds(i * 128, 128)
        return [copy(ak_h.bitcast(U32).at[:, cols], ak.at[i, pl.ds(PAD, S // 2)], sem_a.at[0, i]),
                copy(av_h.bitcast(U32).at[:, cols], av.at[i], sem_a.at[1, i]),
                copy(sk_h.bitcast(U32).at[pl.ds(i * HW, HW), :], sk.at[i], sem_a.at[2, i])]

    def row_copy(src, dst, n, i):
        rows = pl.ds(i * BQ // 2, BQ // 2)
        return copy(src.bitcast(U32).at[rows], dst.at[rows], sem_x.at[n, i])

    def weight_copies(j):
        slot = j & 1
        cps = [copy(src.bitcast(U32).at[:, j, :], dst.at[slot], sem_w.at[slot, n])
               for n, (src, dst) in enumerate([(wq_h, wq), (wuk_h, wk), (wuv_h, wv)])]
        return cps + [copy(wo_h.bitcast(U32).at[j], wo.at[slot], sem_w.at[slot, 3])]

    def head_pair(j):
        slot = j & 1
        ti = j >> 1
        zero = zero_ref[...]
        causal = (jax.lax.broadcasted_iota(jnp.int32, (128, 128), 1) <=
                  jax.lax.broadcasted_iota(jnp.int32, (128, 128), 0))
        issued = []

        def token(lag):
            return zero & pltpu.bitcast(issued[max(len(issued) - lag, 0)][0:8, :], U32)

        def after(v, tok):
            return pltpu.bitcast(pltpu.bitcast(v, U32) | tok, F32)

        k_spec, x_spec, kv, y_spec = {}, {}, {}, {}

        def transform_filter(m):
            k_spec[m] = _mm_nt(_bf(dft[slot, 0]), _bf(sk[ti, :, _tile(m)]))
            return k_spec[m]

        def transform_input(n):
            r0 = PAD + n * HW
            w0, w1, w2 = (ak[ti, r0 - d:r0 - d + HW, :] for d in range(3))
            tok = token(KV_LAG)
            s0, s1, s2, s3 = (
                jnp.concatenate([after(jnp.broadcast_to(shift32[ti, d:d + 1, :], (8, 128)), tok)] * (HW // 8), axis=0)
                for d in range(4))
            e0, o0, e1, o1, o2 = _lo(w0), _hi(w0), _lo(w1), _hi(w1), _hi(w2)
            v = av[ti, _half(n), :]
            kv[n] = jnp.concatenate([(e0 * s0 + o1 * s1 + e1 * s2 + o2 * s3) * _lo(v),
                                     (o0 * s0 + e0 * s1 + o1 * s2 + e1 * s3) * _hi(v)], axis=0)
            x_spec[n] = _mm(_bf(dft[slot, 1]), kv[n].astype(BF))
            return x_spec[n]

        def spectral_product():
            for r in range(HF // 8):
                re, im = slice(r * 8, r * 8 + 8), slice(HF + r * 8, HF + r * 8 + 8)
                for b in range(NC // MB):
                    acc_re, acc_im = [None] * MB, [None] * MB
                    for n in range((b + 1) * MB):
                        tok = yield
                        xr, xi = after(x_spec[n][re, :], tok), after(x_spec[n][im, :], tok)
                        for u in range(MB):
                            m = b * MB + u - n
                            if m >= 0:
                                kr, ki = k_spec[m][re, :], k_spec[m][im, :]
                                pr, pi = xr * kr - xi * ki, xr * ki + xi * kr
                                acc_re[u] = pr if n == 0 else acc_re[u] + pr
                                acc_im[u] = pi if n == 0 else acc_im[u] + pi
                                y_spec[(b * MB + u, r)] = (acc_re[u], acc_im[u])
                        yield acc_im[MB - 1]

        def transform_back(n):
            cur = [y_spec[(n, r)] for r in range(HF // 8)]
            if n == 0:
                parts = [im for _, im in cur] + [-re for re, _ in cur]
            else:
                old = [y_spec[(n - 1, r)] for r in range(HF // 8)]
                parts = [o[0] + v[1] for o, v in zip(old, cur)] + [o[1] - v[0] for o, v in zip(old, cur)]
            conv = _mm(_bf(dft[slot, 2]), jnp.concatenate(parts, axis=0).astype(BF))
            y = conv + kv[n] * ssmd32[pl.ds(ti, 1), :] + jnp.where(slot == 1, y_half[_tile(n), :], 0.0)
            y_half[_tile(n), :] = y
            y_buf[_half(n), pl.ds(pl.multiple_of(ti * 128, 128), 128)] = _pack(y[0:HW, :], y[HW:, :])
            return conv

        qs, ks, vs, ctx, rhs = {}, {}, {}, {}, {}

        def project(i, name):
            src, sums, nt, w = {"q": (x, x_sums, NT // 2, wq), "k": (c, c_sums, NTC // 2, wk),
                                "v": (c, c_sums, NTC // 2, wv)}[name]
            m = [None] * 7

            def step(n, t):
                if (name, t) not in rhs:
                    top, bot = w[slot, _tile(t), :], w[slot, _tile(t + nt), :]
                    rhs[(name, t)] = [v.astype(BF) for v in _rhs_terms(_lo(top), _hi(top), _lo(bot), _hi(bot))]
                if n in LHS_PLAIN:
                    h = LHS_PLAIN[n] // 3
                    lhs = src[_half(2 * i + h), _tile(t + h * nt)]
                else:
                    lhs = sums[LHS_SUMS.index(n), _half(i), _tile(t)]
                d = _mm(_bf(lhs), rhs[(name, t)][n])
                m[n] = d if t == 0 else m[n] + d
                if n == ORDER[-1] and t == nt - 1:
                    c11, c12, c21, c22 = _combine(m)
                    for e, (top, bot) in enumerate([(c11, c21), (c12, c22)]):
                        if name == "q":
                            top, bot = (top * QSCALE).astype(BF), (bot * QSCALE).astype(BF)
                            qs[(e, i, 0)] = jnp.concatenate([top, bot], axis=0)
                            qs[(e, i, 1)] = bot
                        else:
                            dst = ks if name == "k" else vs
                            dst[(e, 2 * i)], dst[(e, 2 * i + 1)] = top.astype(BF), bot.astype(BF)
                return d
            return [P(step, n, t) for n in ORDER for t in range(nt)]

        def key_tiles(i):
            return [(0, t) for t in range(2 * i + 1)] + [(1, 2 * i + 1)]

        def scores(i, e, st):
            def step(u0, t):
                s = _mm_nt(qs[(e, i, u0)], ks[(e, t)])
                for u in range(u0, 2):
                    part = s[_tile(u - u0), :]
                    if t == 2 * i + u:
                        part = jnp.where(causal, part, MASKED)
                    st["s"][(u, t)] = part
                    st["max"][u] = part if t == 0 else jnp.maximum(st["max"][u], part)
                    if t == 2 * i + u:
                        st["max"][u] = jnp.max(st["max"][u], axis=1, keepdims=True)
                return s
            return [P(step, u0, t) for u0, t in key_tiles(i)]

        def attend(i, e, st):
            def step(u0, t):
                tok = token(EXP_LAG) if 2 * i + e >= PACED_FROM else None
                probs = []
                for u in range(u0, 2):
                    m = st["max"][u]
                    if tok is not None:
                        m = jnp.broadcast_to(m, (128, 128))
                        m = jnp.concatenate([after(m[8 * n:8 * n + 8, :], tok) for n in range(16)], axis=0)
                    p = jnp.exp2(st["s"].pop((u, t)) - m)
                    st["sum"][u] = p if t == 0 else st["sum"][u] + p
                    probs.append(p.astype(BF))
                d = _mm(jnp.concatenate(probs, axis=0), vs[(e, t)])
                for u in range(u0, 2):
                    part = d[_tile(u - u0), :]
                    st["out"][u] = part if t == 0 else st["out"][u] + part
                if u0 == 1:
                    for u in range(2):
                        total = jnp.sum(st["sum"][u], axis=1, keepdims=True)
                        r = pl.reciprocal(total, approx=True)
                        ctx[(e, i, u)] = st["out"][u] * (r * (2.0 - total * r))
                return d
            return [P(step, u0, t) for u0, t in key_tiles(i)]

        def project_out(i):
            lhs = []

            def step(t, n):
                left, right = _tile(t), _tile(t + NT // 2)
                if ("o", t) not in rhs:
                    rhs[("o", t)] = _word_terms(_rhs_terms, RHS_PLAIN, *[
                        wo[slot, _half(e), cols] for e in range(2) for cols in (left, right)])
                if not lhs:
                    lhs.extend(v.astype(BF) for v in _lhs_terms(
                        ctx[(0, i, 0)], ctx[(1, i, 0)], ctx[(0, i, 1)], ctx[(1, i, 1)]))
                d = _mm(lhs[n], _bf(rhs[("o", t)][n]))
                acc[n, _tile(i), left] += d
                return d
            return [P(step, t, n) for t in range(NT // 2) for n in ORDER]

        units = [(i, e) for i in range(NB) for e in range(2)]
        states = [dict(s={}, max=[None] * 2, sum=[None] * 2, out=[None] * 2) for _ in units]
        extra = {FWD_AT + n: [P(transform_input, k) for k in range(n * NC // FWD_SPAN, (n + 1) * NC // FWD_SPAN)]
                 for n in range(FWD_SPAN)}
        extra[INV_AT] = [P(transform_back, n) for n in range(NC)]
        seq = [P(transform_filter, m) for m in range(NC)]
        seq += project(0, "k") + project(0, "q") + project(0, "v") + scores(*units[0], states[0])
        ends = []
        for n, (i, e) in enumerate(units):
            if n + 1 < len(units):
                seq += scores(*units[n + 1], states[n + 1])
            if i + 1 == NB:
                fill = project_out(i - 2 + e)
            elif e == 0:
                fill = project(i + 1, "q") + project(i + 1, "k")
            else:
                fill = (project_out(i - 2) if i >= 2 else []) + project(i + 1, "v")
            seq += _merge(_merge(fill, extra.get(n, [])), attend(i, e, states[n]))
            ends.append(len(seq))
        seq += project_out(NB - 1)

        product = spectral_product()
        steps = (HF // 8) * sum((b + 1) * MB for b in range(NC // MB))
        lo, hi = ends[FWD_AT + FWD_SPAN - 1], ends[MAC_END]
        done, last = 0, None
        for k, item in enumerate(seq):
            while k >= lo and done < steps and done * (hi - lo) < (k - lo + 1) * steps:
                next(product)
                tok = token(MAC_LAG)
                last = product.send(tok if last is None else tok & pltpu.bitcast(last, U32))
                done += 1
            issued.append(item())

    first = weight_copies(0) + ssm_copies(0) + [
        copy(src, dst, sem_s.at[n]) for n, (src, dst) in enumerate(
            [(shift_h, shift_v), (ssmd_h, ssmd_v), (dft_h, dft)])]
    gate_copy = copy(gate_h, gate_v, sem_s.at[3])
    rows_in = [(i, row_copy(src_h, src, n, i), src, sums) for i in range(NB)
               for n, (src_h, src, sums) in enumerate([(x_h, x, x_sums), (c_h, c, c_sums)])]
    for cp in [gate_copy] + [cp for _, cp, _, _ in rows_in] + first:
        cp.start()
    zero_ref[...] = jnp.zeros((8, 128), U32)
    for t in range(NT):
        ak[t, 0:PAD, :] = jnp.zeros((PAD, 128), U32)
    acc[...] = jnp.zeros(acc.shape, F32)
    y_half[...] = jnp.zeros(y_half.shape, F32)
    for i, cp, src, sums in rows_in:
        cp.wait()
        mid = src.shape[1] // 2
        terms = _word_terms(_lhs_terms, LHS_PLAIN, *[
            src[_half(2 * i + u), cols] for u in range(2) for cols in (slice(0, mid), slice(mid, 2 * mid))])
        for k, n in enumerate(LHS_SUMS):
            sums[k, _half(i), :] = terms[n]
    gate_copy.wait()
    gate = gate_v[...].astype(F32)
    for n in range(S // 128):
        logit = _bf(x[_half(n), _tile(0)]).astype(F32) * gate[0:1, :]
        for t in range(1, NT):
            logit = logit + _bf(x[_half(n), _tile(t)]).astype(F32) * gate[t:t + 1, :]
        gates[_tile(n), :] = jnp.broadcast_to(jax.nn.sigmoid(jnp.sum(logit, axis=1, keepdims=True)), (128, 128))
    for cp in first:
        cp.wait()
    shift = shift_v[...].astype(F32)
    for t in range(NT):
        shift32[t, 0:4, :] = shift[:, _tile(t)]
    ssmd32[...] = ssmd_v[...].astype(F32) * 0.5

    def iteration(j, carry):
        @pl.when(j > 0)
        def _():
            for cp in weight_copies(j):
                cp.wait()

            @pl.when((j & 1) == 0)
            def _():
                for cp in ssm_copies(j >> 1):
                    cp.wait()

        @pl.when(j + 1 < NP)
        def _():
            for cp in weight_copies(j + 1):
                cp.start()

            @pl.when((j & 1) == 1)
            def _():
                for cp in ssm_copies((j >> 1) + 1):
                    cp.start()

        head_pair(j)
        return carry

    jax.lax.fori_loop(0, NP, iteration, 0)

    stores = []
    for i in range(NB):
        for t in range(NT // 2):
            blocks = [(u, col) for u in range(2) for col in (t, t + NT // 2)]
            for (u, col), b in zip(blocks, _combine([acc[n, _tile(i), _tile(t)] for n in range(7)])):
                g = gates[_tile(2 * i + u), :]
                a = _bf(x[_half(2 * i + u), _tile(col)]).astype(F32) * _bf(y_buf[_half(2 * i + u), _tile(col)]).astype(F32)
                out_v[_tile(2 * i + u), _tile(col)] = (g * a + (1.0 - g) * b).astype(BF)
        stores.append(copy(out_v.at[pl.ds(i * BQ, BQ)], out_h.at[pl.ds(i * BQ, BQ)], sem_o.at[i]))
        stores[-1].start()
    for cp in stores:
        cp.wait()


@jax.jit
def pallas_gated_mix__ssm_conv_h3__compressed_kv_cla__prompt_kernel(
        A_q, A_k, A_v, A_shift_k, A_ssm_k, A_ssm_D, B_x, B_c_kv, B_w_q, B_w_uk, B_w_uv, B_w_o, gate_w):
    del B_x
    vmem, dma = pltpu.VMEM, pltpu.SemaphoreType.DMA
    scratch = [
        vmem((NT, PAD + S // 2, 128), U32), vmem((NT, S // 2, 128), U32),
        vmem((NT, HW, S), U32),
        vmem((S // 2, D), U32), vmem((S // 2, DC), U32),
        vmem((5, NB * HW, D // 2), U32), vmem((5, NB * HW, DC // 2), U32),
        vmem((2, D, HD), U32), vmem((2, DC, HD), U32), vmem((2, DC, HD), U32), vmem((2, HD, D), U32),
        vmem((S, 128), F32), vmem((S // 2, D), U32), vmem((7, S // 2, D // 2), F32), vmem((S, D), BF), vmem((S, 128), F32),
        vmem((4, D), BF), vmem((NT, 128), BF), vmem((NT, 128), BF), vmem((NT, 8, 128), F32), vmem((NT, 128), F32),
        vmem((2, 3, HF, C), U32), vmem((8, 128), U32),
        dma((3, NT)), dma((2, NB)), dma((2, 4)), dma((4,)), dma((NB,)),
    ]
    out = pl.pallas_call(
        _kernel,
        out_shape=jax.ShapeDtypeStruct((S, D), BF),
        in_specs=[pl.BlockSpec(memory_space=pl.ANY)] * 13,
        out_specs=pl.BlockSpec(memory_space=pl.ANY),
        scratch_shapes=scratch,
        compiler_params=pltpu.CompilerParams(vmem_limit_bytes=110 * 1024 * 1024, disable_bounds_checks=True),
    )(A_q.reshape(S, D), A_k.reshape(S, D), A_v.reshape(S, D), A_shift_k.T, A_ssm_k, A_ssm_D.reshape(NT, 128),
      B_c_kv.reshape(S, DC), B_w_q, B_w_uk, B_w_uv, B_w_o.reshape(NP, 2 * HD, D),
      gate_w.reshape(NT, 128), jnp.asarray(_DFT))
    return out.reshape(1, S, D)
```

```python
import functools

import numpy as np
import jax
import jax.numpy as jnp
import jax.experimental.pallas as pl
import jax.experimental.pallas.tpu as pltpu

S, D, H, HD, DC = 2048, 1024, 32, 128, 512
NT, NTC = D // 128, DC // 128
NP = H // 2
BQ = 256
NB = S // BQ
HW = 64
C = 128
NC = S // C
HF = C // 2
MB = 4
PAD = 8

FWD_AT = 2
OUT_AT = [5, 7, 9, 11, 13, 14, 15]
FWD_SPAN = 3
MAC_END = 10
INV_AT = 12
PACED_FROM = 12
MAC_LAG = 18
KV_LAG = 20
EXP_LAG = 6
ORDER = [6, 0, 3, 4, 2, 1, 5]

LOG2E = 1.4426950408889634
QSCALE = (HD ** -0.5) * LOG2E
MASKED = -1e9 * LOG2E
BF, F32, U32 = jnp.bfloat16, jnp.float32, jnp.uint32


def _dft_words():
    t_nat = np.arange(C, dtype=np.float64)
    t_par = np.concatenate([t_nat[0::2], t_nat[1::2]])
    mats = []
    for h in range(2):
        f = 2.0 * np.arange(h * HF, (h + 1) * HF, dtype=np.float64) + 0.5
        row = []
        for t in (t_nat, t_par):
            ang = 2.0 * np.pi * np.outer(f, t) / (2 * C)
            row.append(np.concatenate([np.cos(ang), -np.sin(ang)], axis=0))
        ang = 2.0 * np.pi * np.outer(t_par + C, f) / (2 * C)
        row.append(np.concatenate([np.cos(ang), -np.sin(ang)], axis=1) / C)
        mats.append(np.stack(row))
    bits = np.stack(mats).astype(np.float32).view(np.uint32)
    bits = (bits + np.uint32(0x7FFF) + ((bits >> np.uint32(16)) & np.uint32(1))) >> np.uint32(16)
    return (bits[:, :, 0::2, :] | (bits[:, :, 1::2, :] << np.uint32(16))).astype(np.uint32)


_DFT = _dft_words()


def _mm(a, b):
    return jnp.dot(a, b, preferred_element_type=F32)


def _mm_nt(a, b):
    return jax.lax.dot_general(a, b, (((1,), (1,)), ((), ())), preferred_element_type=F32)


def _bf(words):
    return pltpu.bitcast(words, BF)


def _lo(words):
    return pltpu.bitcast(words << 16, F32)


def _hi(words):
    return pltpu.bitcast(words & jnp.uint32(0xFFFF0000), F32)


def _pack(even_rows, odd_rows):
    return pltpu.pack_elementwise([even_rows, odd_rows], packed_dtype=BF)


def _lhs_terms(a11, a12, a21, a22):
    return [a11 + a22, a21 + a22, a11, a22, a11 + a12, a21 - a11, a12 - a22]


def _rhs_terms(b11, b12, b21, b22):
    return [b11 + b22, b11, b12 - b22, b21 - b11, b22, b11 + b12, b21 + b22]


def _combine(m):
    return m[0] + m[3] - m[4] + m[6], m[2] + m[4], m[1] + m[3], m[0] - m[1] + m[2] + m[5]


LHS_PLAIN = {2: 0, 3: 3}
RHS_PLAIN = {1: 0, 4: 3}
LHS_SUMS = [n for n in range(7) if n not in LHS_PLAIN]


def _word_terms(terms, plain, *words):
    lo, hi = terms(*[_lo(w) for w in words]), terms(*[_hi(w) for w in words])
    return [words[plain[n]] if n in plain else _pack(lo[n], hi[n]) for n in range(7)]


def _merge(a, b):
    out, i, k = [], 0, 0
    while i < len(a) or k < len(b):
        if k >= len(b) or (i < len(a) and (i + 1) * len(b) <= (k + 1) * len(a)):
            out.append(a[i])
            i += 1
        else:
            out.append(b[k])
            k += 1
    return out


def _tile(n):
    return slice(n * 128, (n + 1) * 128)


def _half(n):
    return slice(n * HW, (n + 1) * HW)


def _kernel(x_h, ak_h, av_h, shift_h, sk_h, ssmd_h, c_h, wq_h, wuk_h, wuv_h, wo_h, gate_h, dft_h, out_h,
            ak, av, sk, x, c, x_sums, c_sums, wq, wk, wv, wo, y_half, y_buf, acc, out_v, gates,
            shift_v, ssmd_v, gate_v, shift32, ssmd32, dft, zero_ref,
            sem_a, sem_x, sem_w, sem_s, sem_o):
    P = functools.partial
    copy = pltpu.make_async_copy

    def ssm_copies(i):
        cols = pl.ds(i * 128, 128)
        return [copy(ak_h.bitcast(U32).at[:, cols], ak.at[i, pl.ds(PAD, S // 2)], sem_a.at[0, i]),
                copy(av_h.bitcast(U32).at[:, cols], av.at[i], sem_a.at[1, i]),
                copy(sk_h.bitcast(U32).at[pl.ds(i * HW, HW), :], sk.at[i], sem_a.at[2, i])]

    def row_copy(src, dst, n, i):
        rows = pl.ds(i * BQ // 2, BQ // 2)
        return copy(src.bitcast(U32).at[rows], dst.at[rows], sem_x.at[n, i])

    def weight_copies(j):
        slot = j & 1
        cps = [copy(src.bitcast(U32).at[:, j, :], dst.at[slot], sem_w.at[slot, n])
               for n, (src, dst) in enumerate([(wq_h, wq), (wuk_h, wk), (wuv_h, wv)])]
        return cps + [copy(wo_h.bitcast(U32).at[j], wo.at[slot], sem_w.at[slot, 3])]

    def head_pair(j):
        slot = j & 1
        ti = j >> 1
        zero = zero_ref[...]
        causal = (jax.lax.broadcasted_iota(jnp.int32, (128, 128), 1) <=
                  jax.lax.broadcasted_iota(jnp.int32, (128, 128), 0))
        issued = []

        def token(lag):
            return zero & pltpu.bitcast(issued[max(len(issued) - lag, 0)][0:8, :], U32)

        def after(v, tok):
            return pltpu.bitcast(pltpu.bitcast(v, U32) | tok, F32)

        k_spec, x_spec, kv, y_spec = {}, {}, {}, {}

        def transform_filter(m):
            k_spec[m] = _mm_nt(_bf(dft[slot, 0]), _bf(sk[ti, :, _tile(m)]))
            return k_spec[m]

        def transform_input(n):
            r0 = PAD + n * HW
            w0, w1, w2 = (ak[ti, r0 - d:r0 - d + HW, :] for d in range(3))
            tok = token(KV_LAG)
            s0, s1, s2, s3 = (
                jnp.concatenate([after(jnp.broadcast_to(shift32[ti, d:d + 1, :], (8, 128)), tok)] * (HW // 8), axis=0)
                for d in range(4))
            e0, o0, e1, o1, o2 = _lo(w0), _hi(w0), _lo(w1), _hi(w1), _hi(w2)
            v = av[ti, _half(n), :]
            kv[n] = jnp.concatenate([(e0 * s0 + o1 * s1 + e1 * s2 + o2 * s3) * _lo(v),
                                     (o0 * s0 + e0 * s1 + o1 * s2 + e1 * s3) * _hi(v)], axis=0)
            x_spec[n] = _mm(_bf(dft[slot, 1]), kv[n].astype(BF))
            return x_spec[n]

        def spectral_product():
            for r in range(HF // 8):
                re, im = slice(r * 8, r * 8 + 8), slice(HF + r * 8, HF + r * 8 + 8)
                for b in range(NC // MB):
                    acc_re, acc_im = [None] * MB, [None] * MB
                    for n in range((b + 1) * MB):
                        tok = yield
                        xr, xi = after(x_spec[n][re, :], tok), after(x_spec[n][im, :], tok)
                        for u in range(MB):
                            m = b * MB + u - n
                            if m >= 0:
                                kr, ki = k_spec[m][re, :], k_spec[m][im, :]
                                pr, pi = xr * kr - xi * ki, xr * ki + xi * kr
                                acc_re[u] = pr if n == 0 else acc_re[u] + pr
                                acc_im[u] = pi if n == 0 else acc_im[u] + pi
                                y_spec[(b * MB + u, r)] = (acc_re[u], acc_im[u])
                        yield acc_im[MB - 1]

        def transform_back(n):
            cur = [y_spec[(n, r)] for r in range(HF // 8)]
            if n == 0:
                parts = [im for _, im in cur] + [-re for re, _ in cur]
            else:
                old = [y_spec[(n - 1, r)] for r in range(HF // 8)]
                parts = [o[0] + v[1] for o, v in zip(old, cur)] + [o[1] - v[0] for o, v in zip(old, cur)]
            conv = _mm(_bf(dft[slot, 2]), jnp.concatenate(parts, axis=0).astype(BF))
            y = conv + kv[n] * ssmd32[pl.ds(ti, 1), :] + jnp.where(slot == 1, y_half[_tile(n), :], 0.0)
            y_half[_tile(n), :] = y
            y_buf[_half(n), pl.ds(pl.multiple_of(ti * 128, 128), 128)] = _pack(y[0:HW, :], y[HW:, :])
            return conv

        qs, ks, vs, ctx, rhs = {}, {}, {}, {}, {}

        def project(i, name):
            src, sums, nt, w = {"q": (x, x_sums, NT // 2, wq), "k": (c, c_sums, NTC // 2, wk),
                                "v": (c, c_sums, NTC // 2, wv)}[name]
            m = [None] * 7

            def step(n, t):
                if (name, t) not in rhs:
                    top, bot = w[slot, _tile(t), :], w[slot, _tile(t + nt), :]
                    rhs[(name, t)] = [v.astype(BF) for v in _rhs_terms(_lo(top), _hi(top), _lo(bot), _hi(bot))]
                if n in LHS_PLAIN:
                    h = LHS_PLAIN[n] // 3
                    lhs = src[_half(2 * i + h), _tile(t + h * nt)]
                else:
                    lhs = sums[LHS_SUMS.index(n), _half(i), _tile(t)]
                d = _mm(_bf(lhs), rhs[(name, t)][n])
                m[n] = d if t == 0 else m[n] + d
                if n == ORDER[-1] and t == nt - 1:
                    c11, c12, c21, c22 = _combine(m)
                    for e, (top, bot) in enumerate([(c11, c21), (c12, c22)]):
                        if name == "q":
                            top, bot = (top * QSCALE).astype(BF), (bot * QSCALE).astype(BF)
                            qs[(e, i, 0)] = jnp.concatenate([top, bot], axis=0)
                            qs[(e, i, 1)] = bot
                        else:
                            dst = ks if name == "k" else vs
                            dst[(e, 2 * i)], dst[(e, 2 * i + 1)] = top.astype(BF), bot.astype(BF)
                return d
            return [P(step, n, t) for n in ORDER for t in range(nt)]

        def key_tiles(i):
            return [(0, t) for t in range(2 * i + 1)] + [(1, 2 * i + 1)]

        def scores(i, e, st):
            def step(u0, t):
                s = _mm_nt(qs[(e, i, u0)], ks[(e, t)])
                for u in range(u0, 2):
                    part = s[_tile(u - u0), :]
                    if t == 2 * i + u:
                        part = jnp.where(causal, part, MASKED)
                    st["s"][(u, t)] = part
                    st["max"][u] = part if t == 0 else jnp.maximum(st["max"][u], part)
                    if t == 2 * i + u:
                        st["max"][u] = jnp.max(st["max"][u], axis=1, keepdims=True)
                return s
            return [P(step, u0, t) for u0, t in key_tiles(i)]

        def attend(i, e, st):
            def step(u0, t):
                tok = token(EXP_LAG) if 2 * i + e >= PACED_FROM else None
                probs = []
                for u in range(u0, 2):
                    m = st["max"][u]
                    if tok is not None:
                        m = jnp.broadcast_to(m, (128, 128))
                        m = jnp.concatenate([after(m[8 * n:8 * n + 8, :], tok) for n in range(16)], axis=0)
                    p = jnp.exp2(st["s"].pop((u, t)) - m)
                    st["sum"][u] = p if t == 0 else st["sum"][u] + p
                    probs.append(p.astype(BF))
                d = _mm(jnp.concatenate(probs, axis=0), vs[(e, t)])
                for u in range(u0, 2):
                    part = d[_tile(u - u0), :]
                    st["out"][u] = part if t == 0 else st["out"][u] + part
                if u0 == 1:
                    for u in range(2):
                        total = jnp.sum(st["sum"][u], axis=1, keepdims=True)
                        r = pl.reciprocal(total, approx=True)
                        ctx[(e, i, u)] = st["out"][u] * (r * (2.0 - total * r))
                return d
            return [P(step, u0, t) for u0, t in key_tiles(i)]

        def project_out(i):
            lhs = []

            def step(t, n):
                left, right = _tile(t), _tile(t + NT // 2)
                if ("o", t) not in rhs:
                    rhs[("o", t)] = _word_terms(_rhs_terms, RHS_PLAIN, *[
                        wo[slot, _half(e), cols] for e in range(2) for cols in (left, right)])
                if not lhs:
                    lhs.extend(v.astype(BF) for v in _lhs_terms(
                        ctx[(0, i, 0)], ctx[(1, i, 0)], ctx[(0, i, 1)], ctx[(1, i, 1)]))
                d = _mm(lhs[n], _bf(rhs[("o", t)][n]))
                acc[n, _tile(i), left] += d
                return d
            return [P(step, t, n) for t in range(NT // 2) for n in ORDER]

        units = [(i, e) for i in range(NB) for e in range(2)]
        states = [dict(s={}, max=[None] * 2, sum=[None] * 2, out=[None] * 2) for _ in units]
        extra = {FWD_AT + n: [P(transform_input, k) for k in range(n * NC // FWD_SPAN, (n + 1) * NC // FWD_SPAN)]
                 for n in range(FWD_SPAN)}
        extra[INV_AT] = [P(transform_back, n) for n in range(NC)]
        seq = [P(transform_filter, m) for m in range(NC)]
        seq += project(0, "k") + project(0, "q") + project(0, "v") + scores(*units[0], states[0])
        ends = []
        for n, (i, e) in enumerate(units):
            ahead = scores(*units[n + 1], states[n + 1]) if n + 1 < len(units) else []
            fill = []
            if i + 1 < NB:
                fill += project(i + 1, "v") if e else project(i + 1, "q") + project(i + 1, "k")
            if n in OUT_AT:
                fill += project_out(OUT_AT.index(n))
            fill = _merge(fill, extra.get(n, []))
            seq += _merge(fill, ahead + attend(i, e, states[n]))
            ends.append(len(seq))
        seq += project_out(NB - 1)

        product = spectral_product()
        steps = (HF // 8) * sum((b + 1) * MB for b in range(NC // MB))
        lo, hi = ends[FWD_AT + FWD_SPAN - 1], ends[MAC_END]
        done, last = 0, None
        for k, item in enumerate(seq):
            while k >= lo and done < steps and done * (hi - lo) < (k - lo + 1) * steps:
                next(product)
                tok = token(MAC_LAG)
                last = product.send(tok if last is None else tok & pltpu.bitcast(last, U32))
                done += 1
            issued.append(item())

    first = weight_copies(0) + ssm_copies(0) + [
        copy(src, dst, sem_s.at[n]) for n, (src, dst) in enumerate(
            [(shift_h, shift_v), (ssmd_h, ssmd_v), (dft_h, dft)])]
    gate_copy = copy(gate_h, gate_v, sem_s.at[3])
    rows_in = [(i, row_copy(src_h, src, n, i), src, sums) for i in range(NB)
               for n, (src_h, src, sums) in enumerate([(x_h, x, x_sums), (c_h, c, c_sums)])]
    for cp in [gate_copy] + [cp for _, cp, _, _ in rows_in] + first:
        cp.start()
    zero_ref[...] = jnp.zeros((8, 128), U32)
    for t in range(NT):
        ak[t, 0:PAD, :] = jnp.zeros((PAD, 128), U32)
    acc[...] = jnp.zeros(acc.shape, F32)
    y_half[...] = jnp.zeros(y_half.shape, F32)
    for i, cp, src, sums in rows_in:
        cp.wait()
        mid = src.shape[1] // 2
        terms = _word_terms(_lhs_terms, LHS_PLAIN, *[
            src[_half(2 * i + u), cols] for u in range(2) for cols in (slice(0, mid), slice(mid, 2 * mid))])
        for k, n in enumerate(LHS_SUMS):
            sums[k, _half(i), :] = terms[n]
    gate_copy.wait()
    gate = gate_v[...].astype(F32)
    for n in range(S // 128):
        logit = _bf(x[_half(n), _tile(0)]).astype(F32) * gate[0:1, :]
        for t in range(1, NT):
            logit = logit + _bf(x[_half(n), _tile(t)]).astype(F32) * gate[t:t + 1, :]
        gates[_tile(n), :] = jnp.broadcast_to(jax.nn.sigmoid(jnp.sum(logit, axis=1, keepdims=True)), (128, 128))
    for cp in first:
        cp.wait()
    shift = shift_v[...].astype(F32)
    for t in range(NT):
        shift32[t, 0:4, :] = shift[:, _tile(t)]
    ssmd32[...] = ssmd_v[...].astype(F32) * 0.5

    def iteration(j, carry):
        @pl.when(j > 0)
        def _():
            for cp in weight_copies(j):
                cp.wait()

            @pl.when((j & 1) == 0)
            def _():
                for cp in ssm_copies(j >> 1):
                    cp.wait()

        @pl.when(j + 1 < NP)
        def _():
            for cp in weight_copies(j + 1):
                cp.start()

            @pl.when((j & 1) == 1)
            def _():
                for cp in ssm_copies((j >> 1) + 1):
                    cp.start()

        head_pair(j)
        return carry

    jax.lax.fori_loop(0, NP, iteration, 0)

    stores = []
    for i in range(NB):
        for t in range(NT // 2):
            blocks = [(u, col) for u in range(2) for col in (t, t + NT // 2)]
            for (u, col), b in zip(blocks, _combine([acc[n, _tile(i), _tile(t)] for n in range(7)])):
                g = gates[_tile(2 * i + u), :]
                a = _bf(x[_half(2 * i + u), _tile(col)]).astype(F32) * _bf(y_buf[_half(2 * i + u), _tile(col)]).astype(F32)
                out_v[_tile(2 * i + u), _tile(col)] = (g * a + (1.0 - g) * b).astype(BF)
        stores.append(copy(out_v.at[pl.ds(i * BQ, BQ)], out_h.at[pl.ds(i * BQ, BQ)], sem_o.at[i]))
        stores[-1].start()
    for cp in stores:
        cp.wait()


@jax.jit
def pallas_gated_mix__ssm_conv_h3__compressed_kv_cla__prompt_kernel(
        A_q, A_k, A_v, A_shift_k, A_ssm_k, A_ssm_D, B_x, B_c_kv, B_w_q, B_w_uk, B_w_uv, B_w_o, gate_w):
    del B_x
    vmem, dma = pltpu.VMEM, pltpu.SemaphoreType.DMA
    scratch = [
        vmem((NT, PAD + S // 2, 128), U32), vmem((NT, S // 2, 128), U32),
        vmem((NT, HW, S), U32),
        vmem((S // 2, D), U32), vmem((S // 2, DC), U32),
        vmem((5, NB * HW, D // 2), U32), vmem((5, NB * HW, DC // 2), U32),
        vmem((2, D, HD), U32), vmem((2, DC, HD), U32), vmem((2, DC, HD), U32), vmem((2, HD, D), U32),
        vmem((S, 128), F32), vmem((S // 2, D), U32), vmem((7, S // 2, D // 2), F32), vmem((S, D), BF), vmem((S, 128), F32),
        vmem((4, D), BF), vmem((NT, 128), BF), vmem((NT, 128), BF), vmem((NT, 8, 128), F32), vmem((NT, 128), F32),
        vmem((2, 3, HF, C), U32), vmem((8, 128), U32),
        dma((3, NT)), dma((2, NB)), dma((2, 4)), dma((4,)), dma((NB,)),
    ]
    out = pl.pallas_call(
        _kernel,
        out_shape=jax.ShapeDtypeStruct((S, D), BF),
        in_specs=[pl.BlockSpec(memory_space=pl.ANY)] * 13,
        out_specs=pl.BlockSpec(memory_space=pl.ANY),
        scratch_shapes=scratch,
        compiler_params=pltpu.CompilerParams(vmem_limit_bytes=110 * 1024 * 1024, disable_bounds_checks=True),
    )(A_q.reshape(S, D), A_k.reshape(S, D), A_v.reshape(S, D), A_shift_k.T, A_ssm_k, A_ssm_D.reshape(NT, 128),
      B_c_kv.reshape(S, DC), B_w_q, B_w_uk, B_w_uv, B_w_o.reshape(NP, 2 * HD, D),
      gate_w.reshape(NT, 128), jnp.asarray(_DFT))
    return out.reshape(1, S, D)
```
